```python
import jax
import jax.numpy as jnp

def _softmax(x, axis=-1):
    return jax.nn.softmax(x, axis=axis)
def _gelu(x):
    return jax.nn.gelu(x, approximate=True)
def _silu(x):
    return jax.nn.silu(x)
def _sigmoid(x):
    return jax.nn.sigmoid(x)
def _layernorm(x, axis=-1, eps=1e-5):
    m = jnp.mean(x, axis=axis, keepdims=True)
    v = jnp.var(x, axis=axis, keepdims=True)
    return (x - m) / jnp.sqrt(v + eps)
def _scatter_add(tgt, idx, src, axis=0):
    return tgt.at[idx].add(src)
def _segment_sum(src, seg, n):
    return jax.ops.segment_sum(src, seg, n)
class _Rng:
    def __init__(self, key):
        self._k = key
    def _next(self):
        self._k, sub = jax.random.split(self._k)
        return sub
    def normal(self, shape):
        return jax.random.normal(self._next(), shape, dtype=jnp.bfloat16)
    def randint(self, lo, hi, shape):
        return jax.random.randint(self._next(), shape, lo, hi, dtype=jnp.int32)
    def uniform(self, shape, lo=0.0, hi=1.0):
        return jax.random.uniform(self._next(), shape, jnp.bfloat16, lo, hi)
    def permutation(self, n):
        return jax.random.permutation(self._next(), n)


kernel_name = 'gated_mix__sliding_local_dilated__moe_arch_mod__prompt'

def setup_inputs():
    _rng = _Rng(jax.random.key(int.from_bytes(__import__("os").urandom(4), "little")))
    _w = (lambda a: (lambda t: t.astype(jnp.bfloat16) if jnp.issubdtype(t.dtype, jnp.floating) else t)(jnp.asarray(a)))
    def _A_setup():
        B, S, D = 1, 2048, 640
        return {
            "x": _w((lambda *s: _rng.normal(s) * 0.05)(B, S, D)),
            "wqkv": _w((lambda *s: _rng.normal(s) * 0.05)(D, 3 * D)),
            "wo": _w((lambda *s: _rng.normal(s) * 0.05)(D, D)),
        }
    _A_in = _A_setup()

    def _B_setup():
        B, S, D, F, C = 1, 2048, 640, 1728, 2
        return {
            "x": _w((lambda *s: _rng.normal(s) * 0.05)(B, S, D)),
            "w_r": _w((lambda *s: _rng.normal(s) * 0.05)(D)),
            "w_gate": _w((lambda *s: _rng.normal(s) * 0.05)(D, F)),
            "w_up": _w((lambda *s: _rng.normal(s) * 0.05)(D, F)),
            "w_down": _w((lambda *s: _rng.normal(s) * 0.05)(F, D)),
        }
    _B_in = _B_setup()

    return {
        "A_x": _A_in["x"],
        "A_wqkv": _A_in["wqkv"],
        "A_wo": _A_in["wo"],
        "B_x": _B_in["x"],
        "B_w_r": _B_in["w_r"],
        "B_w_gate": _B_in["w_gate"],
        "B_w_up": _B_in["w_up"],
        "B_w_down": _B_in["w_down"],
        "gate_w": _w((lambda *s: _rng.normal(s) * 0.05)(640)),
    }

def reference(A_x, A_wqkv, A_wo, B_x, B_w_r, B_w_gate, B_w_up, B_w_down, gate_w):
    def _A_ref(x, wqkv, wo):
        B, S, D = x.shape
        H = 32; Dh = D // H
        W, dil = 8, 2
        qkv = (lambda x, *d: x.transpose(*d))((x @ wqkv).reshape(B, S, 3, H, Dh), 2, 0, 3, 1, 4)
        q, k, v = qkv[0], qkv[1], qkv[2]
        scale = Dh ** -0.5
        pos = jnp.arange(S)
        off = jnp.arange(W) * dil
        idx = pos[:, None] - off[None, :]
        mask = idx >= 0
        idx_c = jnp.where(mask, idx, 0).reshape(-1)
        kg = k[:, :, idx_c, :].reshape(B, H, S, W, Dh)
        vg = v[:, :, idx_c, :].reshape(B, H, S, W, Dh)
        logits = jnp.einsum("bhsd,bhswd->bhsw", q, kg) * scale
        logits = jnp.where(mask[None, None, :, :], logits, -1e9)
        attn = _softmax(logits, axis=-1)
        o = jnp.einsum("bhsw,bhswd->bhsd", attn, vg)
        return (lambda x, *d: x.transpose(*d))(o, 0, 2, 1, 3).reshape(B, S, D) @ wo

    def _B_ref(x, w_r, w_gate, w_up, w_down):
        B, S, D = x.shape
        C = 2
        r = x @ w_r
        idx = jnp.argsort(-r, axis=-1)[:, :C]
        idx_e = jnp.repeat(idx.reshape(B, C, 1), D, axis=2)
        x_sel = jnp.take_along_axis(x, idx_e, axis=1)
        g = _silu(x_sel @ w_gate)
        u = x_sel @ w_up
        y = (g * u) @ w_down
        r_sel = _sigmoid(jnp.take_along_axis(r, idx, axis=1))
        y = y * r_sel.reshape(B, C, 1)
        b_off = (jnp.arange(B) * S).reshape(B, 1)
        flat_idx = (idx + b_off).reshape(B * C)
        zero = (x * 0.0).reshape(B * S, D)
        upd = _scatter_add(zero, flat_idx, y.reshape(B * C, D), axis=0)
        return x + upd.reshape(B, S, D)

    x = A_x
    g = _sigmoid((x * gate_w).sum(-1, keepdims=True))
    a = _A_ref(x, A_wqkv, A_wo)
    b = _B_ref(x, B_w_r, B_w_gate, B_w_up, B_w_down)
    return g * a + (1 - g) * b
```

```python
import contextlib
import functools
import itertools
import math

import jax
import jax.numpy as jnp
from jax import lax
import jax.experimental.pallas as pl
import jax.experimental.pallas.tpu as pltpu

CFG = dict(
    flags=None, interpret=False, scopes=False,
    head=([("start", "w0"), ("start", "x0"), ("wait", "w0"), ("start", "w1"), ("w", 0)],
          [("wait", "x0"), ("start", "w2"), ("x", (0,))]),
    events={
        (0, 2): [("wait", "w1"), ("start", "w3"), ("w", 1)],
        (1, 1): [("wait", "w2"), ("start", "x1"), ("w", 2)],
        (2, 0): [("wait", "w3"), ("w", 3)],
        (3, 0): [("wait", "x1"), ("start", "x2"), ("w", 4), ("x", (1,))],
        (4, 0): [("w", 5)],
        (5, 0): [("wait", "x2"), ("start", "wg"), ("start", "wu"), ("gates", (0,))],
        (6, 0): [("gates", (1,))],
        (7, 0): [("x", (2,))],
        (8, 0): [("gates", (2,))],
        (9, 0): [("wait", "wg"), ("wait", "wu"), ("start", "wd"), ("start", "wo"),
                 ("gates", (3,))],
        (10, 0): [("route", ())],
        (11, 0): [("x", (3,))],
        (13, 0): [("wait", "wd"), ("wait", "wo"), ("wo", ())],
    },
    order=lambda s: ((1, s), (2, s - 1), (0, s + 1)),
    cs=((0, 1), (2, 3), (4,)))

S, D, H, F = 2048, 640, 32, 1728
DH = D // H
W = 8
HG = H // 8
GR = 8 * DH
TB = 512
NB = S // TB
NU = TB // 128
NC = D // 128
NE = W - 1
SCALE = DH ** -0.5
EXP_SCALE = SCALE * math.log2(math.e)
MASKED = -1e9 / SCALE

f32, bf16, u32 = jnp.float32, jnp.bfloat16, jnp.uint32
NT = (((1,), (1,)), ((), ()))


def _kernel(x_hbm, wqkv_hbm, wo_hbm, wr_ref, wg_hbm, wu_hbm, wd_hbm, gw_ref,
            out_hbm,
            x_v, wqkv_v, wo_v, wg_v, wu_v, wd_v, out_v,
            tmp, score_s, sems, out_sems):
    n_sem = [0]

    def copy(src, dst):
        c = pltpu.make_async_copy(src, dst, sems.at[n_sem[0]])
        n_sem[0] += 1
        return c

    def start(cps):
        for c in cps:
            c.start()

    def wait(cps):
        for c in cps:
            c.wait()

    def rows(i):
        return pl.ds(pl.multiple_of(i * (TB // 2), TB // 2), TB // 2)

    def lanes(c):
        return pl.ds(c * 128, 128)

    x_hbm, out_hbm, wqkv_hbm, wo_hbm, wg_hbm, wu_hbm, wd_hbm = (
        r.bitcast(u32) for r in (x_hbm, out_hbm, wqkv_hbm, wo_hbm, wg_hbm, wu_hbm, wd_hbm))

    def cp_x(lo, hi):
        rws = pl.ds(lo * (TB // 2), (hi - lo) * (TB // 2))
        return [copy(x_hbm.at[rws, lanes(c)], x_v.at[c, rws]) for c in range(NC)]

    def cp_out(i, c):
        return pltpu.make_async_copy(out_v.at[c, rows(i)], out_hbm.at[rows(i), lanes(c)],
                                     out_sems.at[i, c])

    def slab(i, u):
        return pl.ds(i * (TB // 2) + u, 64, stride=NU)

    def load_rows(ref, rws=slice(None)):
        return jnp.concatenate([ref[c, rws, :] for c in range(ref.shape[0])], axis=1)

    def load_bf16(ref, rws=slice(None)):
        return pltpu.bitcast(load_rows(ref, rws), bf16)

    def store_bf16(ref, rws, val):
        val = pltpu.bitcast(val.astype(bf16), u32)
        for c in range(ref.shape[0]):
            ref[c, rws, :] = val[:, c * 128:(c + 1) * 128]

    def head_major_rows(base, d):
        return pl.ds(base + d, 8, stride=DH)

    wT, woT, xT, gate, oT = {}, {}, {}, {}, {}
    w_ready = set()

    def prep_qkv(p, g):
        base = p * D + g * GR
        for t in range(base // 128, (base + GR - 1) // 128 + 1):
            if t not in w_ready:
                w_ready.add(t)
                for c in range(NC):
                    tmp[c, lanes(t), :] = pltpu.bitcast(
                        wqkv_v[pl.ds(c * 64, 64), lanes(t)], bf16).astype(f32).T
                    yield 60
        parts = []
        for d in range(0, DH, 2):
            two = jnp.concatenate([load_rows(tmp, head_major_rows(base, d)),
                                   load_rows(tmp, head_major_rows(base, d + 1))], axis=0)
            parts.append(two.astype(bf16))
            yield 30
        wT[p, g] = jnp.concatenate(parts, axis=0)

    def prep_wo():
        for c in range(NC):
            perm = jnp.concatenate(
                [wo_v[c, pl.ds(g * GR // 2 + dp, 8, stride=DH // 2), :]
                 for g in range(HG) for dp in range(DH // 2)], axis=0)
            woT[c] = pltpu.bitcast(perm, bf16).T
            yield 200

    def prep_x(i):
        for u in range(NU):
            cols = []
            for c in range(NC):
                cols.append(pltpu.bitcast(x_v[c, slab(i, u), :], bf16).T)
                yield 40
            xT[i, u] = jnp.concatenate(cols, axis=0)

    def gates(i):
        gw = gw_ref[...].astype(f32).reshape(1, D)
        wr = wr_ref[...].astype(f32).reshape(1, D)
        for u in range(NU):
            g_acc = r_acc = None
            for c in range(NC):
                xs = pltpu.bitcast(x_v[c, slab(i, u), :], bf16).astype(f32)
                gp, rp = xs * gw[:, c * 128:(c + 1) * 128], xs * wr[:, c * 128:(c + 1) * 128]
                g_acc = gp if c == 0 else g_acc + gp
                r_acc = rp if c == 0 else r_acc + rp
                yield 80
            gt = jax.nn.sigmoid(jnp.sum(g_acc, axis=1, keepdims=True))
            gate[i, u] = jnp.broadcast_to(gt, (128, 128))
            score_s[pl.ds(i * NU + u, 1), :] = jnp.sum(r_acc.T, axis=0, keepdims=True)
            yield 200

    lane = lax.broadcasted_iota(jnp.int32, (1, 128), 1)
    query, raw, logit, prob, inv, acc = {}, {}, {}, {}, {}, {}

    def taps(p, i, g, t, d, cur):
        prev = raw.pop((p, g, t, d)) if i > 0 else 0.0
        if i + 1 < NB:
            raw[p, g, t, d] = cur
        for wrap in range((W - 1 + NU - 1) // NU + 1):
            us = [u for u in range(NU) if 0 <= u - t + wrap * NU < W]
            if us:
                x = cur if wrap == 0 else pltpu.roll(
                    jnp.where(lane >= 128 - 2 * wrap, prev, cur), 2 * wrap, 1)
                for u in us:
                    yield u, u - t + wrap * NU, x

    def scores(i, g, t, k):
        for d in range(DH):
            for u, w, x in taps(1, i, g, t, d, k[d * 8:(d + 1) * 8]):
                term = query[i, g, u][d * 8:(d + 1) * 8] * x
                logit[u, w] = logit[u, w] + term if d else term

    def softmax(i, g):
        for u in range(NU):
            ls = []
            for w in range(W):
                l = logit.pop((u, w))
                if i == 0 and w > u:
                    l = jnp.where(lane >= 2 * ((w - u + NU - 1) // NU), l, MASKED)
                ls.append(l)
            m = functools.reduce(jnp.maximum, ls)
            for w in range(W):
                prob[u, w] = jnp.exp2((ls[w] - m) * EXP_SCALE)
            inv[u] = 1.0 / functools.reduce(jnp.add, [prob[u, w] for w in range(W)])

    def values(i, g, t, v):
        for d in range(DH):
            for u, w, x in taps(2, i, g, t, d, v[d * 8:(d + 1) * 8]):
                term = prob[u, w] * x
                acc[u, d] = acc[u, d] + term if (u, d) in acc else term
            if t == NU - 1 and d % 2:
                for u in range(NU):
                    pair = [acc.pop((u, d - 1)) * inv[u], acc.pop((u, d)) * inv[u]]
                    oT.setdefault((i, u), []).append(pltpu.bitcast(
                        pltpu.pack_elementwise(pair, packed_dtype=bf16), u32))

    def project(work, t):
        for i in sorted({i for _, i, _ in work}):
            mine = [(p, g) for p, ii, g in work if ii == i]
            r = jnp.dot(jnp.concatenate([wT[pg] for pg in mine], axis=0), xT[i, t],
                        preferred_element_type=f32)
            for n, (p, g) in enumerate(mine):
                part = r[n * GR:(n + 1) * GR]
                if p == 0:
                    query[i, g, t] = part
                else:
                    (scores, values)[p - 1](i, g, t, part)

    jobs = []

    credit = [0]

    def background(budget):
        credit[0] += budget
        while jobs and credit[0] > 0:
            cost = next(jobs[0], None)
            if cost is None:
                jobs.pop(0)
            else:
                credit[0] -= cost
        if not jobs:
            credit[0] = 0

    picks = []

    def route():
        r = score_s[...]
        r = r.astype(bf16).astype(f32)
        key = jnp.where(r != r, -jnp.inf, r)
        sub = lax.broadcasted_iota(jnp.int32, (NB * NU, 128), 0)
        pos = (sub // NU) * TB + (lane // 2) * (2 * NU) + (sub % NU) * 2 + lane % 2
        free = pos >= 0
        for _ in range(2):
            m = jnp.max(jnp.where(free, key, -jnp.inf), keepdims=True)
            idx = jnp.min(jnp.where(free & (key == m), pos, S - 1))
            score = jnp.sum(jnp.where(pos == idx, r, 0.0), keepdims=True)
            free = free & (pos != idx)
            picks.append((idx, jax.nn.sigmoid(score)))
            yield 50

    def ffn():
        row = lax.broadcasted_iota(jnp.int32, (16, D), 0)
        tiles = [pl.ds(pl.multiple_of((idx // 16) * 8, 8), 8) for idx, _ in picks]
        hits = [row == idx % 16 for idx, _ in picks]
        xs = jnp.concatenate(
            [jnp.where(h, load_bf16(x_v, t).astype(f32), 0.0) for t, h in zip(tiles, hits)],
            axis=0).astype(bf16)
        pre = lax.dot_general(xs, pltpu.bitcast(wg_v[...], bf16), NT, preferred_element_type=f32)
        up = lax.dot_general(xs, pltpu.bitcast(wu_v[...], bf16), NT, preferred_element_type=f32)
        h = (pre * jax.nn.sigmoid(pre) * up).astype(bf16)
        y = jnp.dot(h, pltpu.bitcast(wd_v[...], bf16), preferred_element_type=f32)
        for n, (t, hit, (_, wgt)) in enumerate(zip(tiles, hits, picks)):
            cur = load_bf16(x_v, t).astype(f32)
            store_bf16(x_v, t, jnp.where(hit, cur + y[n * 16:(n + 1) * 16] * wgt, cur))

    def emit(i, cs):
        rhs = jnp.concatenate(
            [pltpu.bitcast(jnp.concatenate(oT[i, u], axis=0), bf16) for u in range(NU)], axis=1)
        aT = jnp.dot(jnp.concatenate([woT[c] for c in cs], axis=0), rhs,
                     preferred_element_type=f32)
        for n, c in enumerate(cs):
            for u in range(NU):
                a = aT[n * 128:(n + 1) * 128, u * 128:(u + 1) * 128].T
                b = pltpu.bitcast(x_v[c, slab(i, u), :], bf16).astype(f32)
                gt = gate[i, u]
                o = gt * a + (1.0 - gt) * b
                out_v[c, slab(i, u), :] = pltpu.bitcast(o.astype(bf16), u32)
            cp_out(i, c).start()

    def scope(name):
        return jax.named_scope("@" + name) if CFG["scopes"] else contextlib.nullcontext()

    n_groups = NB * HG
    steps = [[(p, n // HG, n % HG) for p, n in CFG["order"](s) if 0 <= n < n_groups]
             for s in range(-1, n_groups + 1)]

    def w_tiles(work):
        return [t for p, i, g in work
                for t in range((p * D + g * GR) // 128, (p * D + g * GR + GR - 1) // 128 + 1)]

    seen = set()

    def w_batch(lo, hi):
        new = [t for work in steps[lo:hi] for t in w_tiles(work)]
        new = [t for t in dict.fromkeys(new) if t not in seen]
        seen.update(new)
        runs = [[t for _, t in run] for _, run in
                itertools.groupby(enumerate(sorted(new)), lambda nt: nt[1] - nt[0])]
        cols = [pl.ds(run[0] * 128, len(run) * 128) for run in runs]
        return [copy(wqkv_hbm.at[:, cl], wqkv_v.at[:, cl]) for cl in cols]

    batch = dict(w0=w_batch(0, 1), w1=w_batch(1, 2), w2=w_batch(2, 3), w3=w_batch(3, len(steps)),
                 x0=cp_x(0, 1), x1=cp_x(1, 2), x2=cp_x(2, NB),
                 wo=[copy(wo_hbm.at[:, lanes(c)], wo_v.at[c]) for c in range(NC)],
                 wg=[copy(wg_hbm, wg_v)], wu=[copy(wu_hbm, wu_v)], wd=[copy(wd_hbm, wd_v)])
    flying = []

    def run(actions):
        cost = 0
        for act, arg in actions:
            if act == "start":
                start(batch[arg])
                flying.append(arg)
            elif act == "wait":
                wait(batch[arg])
                flying.remove(arg)
            elif act == "w":
                for p, i, g in steps[arg]:
                    if i == 0:
                        jobs.append(prep_qkv(p, g))
                        cost += 700
            else:
                job, c = dict(x=(prep_x, 800), gates=(gates, 2400), wo=(prep_wo, 1000),
                              route=(route, 100))[act]
                jobs.append(job(*arg))
                cost += c
        return cost

    for actions in CFG["head"]:
        run(actions)
        background(1e9)
    for s, work in enumerate(steps):
        with scope(f"s{s}"):
            cost = 0
            for t in range(NU):
                cost += run(CFG["events"].get((s, t), ()))
                project(work, t)
                share = cost / (NU - t)
                background(share)
                cost -= share
            background(1e9)
            for p, i, g in work:
                if p == 1:
                    softmax(i, g)
        if s == CFG.get("stop"):
            out_v[0, 0:8, :] = pltpu.bitcast(functools.reduce(
                jnp.add, list(prob.values()) + list(inv.values()) + [v[:8] for v in query.values()]), u32)
            for ws in oT.values():
                for k, word in enumerate(ws):
                    out_v[1, pl.ds(8 * k, 8), :] = word
            wait([c for nm in flying for c in batch[nm]])
            cp_out(0, 0).start()
            cp_out(0, 0).wait()
            return
    with scope("ffn"):
        ffn()
    for i in range(NB):
        with scope(f"c{i}"):
            for cs in CFG["cs"]:
                emit(i, cs)
    wait([cp_out(i, c) for i in range(NB) for c in range(NC)])


@jax.jit
def pallas_gated_mix__sliding_local_dilated__moe_arch_mod__prompt_kernel(
    A_x: jax.Array,
    A_wqkv: jax.Array,
    A_wo: jax.Array,
    B_x: jax.Array,
    B_w_r: jax.Array,
    B_w_gate: jax.Array,
    B_w_up: jax.Array,
    B_w_down: jax.Array,
    gate_w: jax.Array,
):
    hbm = pl.BlockSpec(memory_space=pl.ANY)
    vmem = pl.BlockSpec(memory_space=pltpu.VMEM)
    return pl.pallas_call(
        _kernel,
        out_shape=jax.ShapeDtypeStruct((S, D), A_x.dtype),
        in_specs=[hbm, hbm, hbm, vmem, hbm, hbm, hbm, vmem],
        out_specs=hbm,
        interpret=CFG["interpret"],
        scratch_shapes=[
            pltpu.VMEM((NC, S // 2, 128), u32),
            pltpu.VMEM((D // 2, 3 * D), u32),
            pltpu.VMEM((NC, D // 2, 128), u32),
            pltpu.VMEM((F // 2, D), u32),
            pltpu.VMEM((F // 2, D), u32),
            pltpu.VMEM((F // 2, D), u32),
            pltpu.VMEM((NC, S // 2, 128), u32),
            pltpu.VMEM((NC, 3 * D, 128), f32),
            pltpu.VMEM((NB * NU, 128), f32),
            pltpu.SemaphoreType.DMA((64,)),
            pltpu.SemaphoreType.DMA((NB, NC)),
        ],
        compiler_params=pltpu.CompilerParams(
            vmem_limit_bytes=100 * 1024 * 1024, flags=CFG["flags"]),
    )(A_x.reshape(S, D), A_wqkv, A_wo, B_w_r, B_w_gate.T, B_w_up.T, B_w_down,
      gate_w).reshape(A_x.shape)
```

```python
import contextlib
import functools
import itertools
import math

import jax
import jax.numpy as jnp
from jax import lax
import jax.experimental.pallas as pl
import jax.experimental.pallas.tpu as pltpu

CFG = dict(
    flags=None, interpret=False, scopes=False,
    head=([("start", "w0"), ("start", "x0"), ("wait", "w0"), ("start", "w1"), ("w", 0)],
          [("wait", "x0"), ("start", "w2"), ("x", (0,))]),
    events={
        (0, 2): [("wait", "w1"), ("start", "w3"), ("w", 1)],
        (1, 1): [("wait", "w2"), ("start", "x1"), ("w", 2)],
        (2, 0): [("wait", "w3"), ("start", "x2"), ("w", 3)],
        (3, 0): [("wait", "x1"), ("w", 4), ("x", (1,))],
        (4, 0): [("wait", "x2"), ("start", "wg"), ("start", "wu"), ("start", "wd"),
                 ("start", "wo"), ("w", 5)],
        (5, 0): [("gates", (0,))],
        (6, 0): [("gates", (1,))],
        (7, 0): [("x", (2,)), ("gates", (2,))],
        (8, 0): [("gates", (3,))],
        (9, 0): [("route", ())],
        (10, 0): [("wait", "wg"), ("wait", "wu"), ("wait", "wd"), ("wait", "wo"),
                  ("hidden", ()), ("out", ())],
        (11, 0): [("x", (3,))],
        (14, 0): [("wo", ())],
    },
    ties=0, lag=3,
    slow={10: 2800, 11: 2400, 12: 2800, 13: 2800, 14: 2400, 15: 2800, 16: 2400, 17: 1200},
    order=lambda s: ((1, s), (2, s - 1), (0, s + 1)),
    cs=((0, 1), (2, 3), (4,)))

S, D, H, F = 2048, 640, 32, 1728
DH = D // H
W = 8
HG = H // 8
GR = 8 * DH
TB = 512
NB = S // TB
NU = TB // 128
NC = D // 128
NE = W - 1
SCALE = DH ** -0.5
EXP_SCALE = SCALE * math.log2(math.e)
MASKED = -1e9 / SCALE

f32, bf16, u32 = jnp.float32, jnp.bfloat16, jnp.uint32
NT = (((1,), (1,)), ((), ()))


def _kernel(x_hbm, wqkv_hbm, wo_hbm, wr_ref, wg_hbm, wu_hbm, wd_hbm, gw_ref,
            out_hbm,
            x_v, wqkv_v, wo_v, wg_v, wu_v, wd_v, out_v,
            tmp, score_s, sems, out_sems):
    n_sem = [0]

    def copy(src, dst):
        c = pltpu.make_async_copy(src, dst, sems.at[n_sem[0]])
        n_sem[0] += 1
        return c

    def start(cps):
        for c in cps:
            c.start()

    def wait(cps):
        for c in cps:
            c.wait()

    def rows(i):
        return pl.ds(pl.multiple_of(i * (TB // 2), TB // 2), TB // 2)

    def lanes(c):
        return pl.ds(c * 128, 128)

    x_hbm, out_hbm, wqkv_hbm, wo_hbm, wg_hbm, wu_hbm, wd_hbm = (
        r.bitcast(u32) for r in (x_hbm, out_hbm, wqkv_hbm, wo_hbm, wg_hbm, wu_hbm, wd_hbm))

    def cp_x(lo, hi):
        rws = pl.ds(lo * (TB // 2), (hi - lo) * (TB // 2))
        return [copy(x_hbm.at[rws, lanes(c)], x_v.at[c, rws]) for c in range(NC)]

    def cp_out(i, c):
        return pltpu.make_async_copy(out_v.at[c, rows(i)], out_hbm.at[rows(i), lanes(c)],
                                     out_sems.at[i, c])

    def slab(i, u):
        return pl.ds(i * (TB // 2) + u, 64, stride=NU)

    def load_rows(ref, rws=slice(None)):
        return jnp.concatenate([ref[c, rws, :] for c in range(ref.shape[0])], axis=1)

    def load_bf16(ref, rws=slice(None)):
        return pltpu.bitcast(load_rows(ref, rws), bf16)

    def store_bf16(ref, rws, val):
        val = pltpu.bitcast(val.astype(bf16), u32)
        for c in range(ref.shape[0]):
            ref[c, rws, :] = val[:, c * 128:(c + 1) * 128]

    def head_major_rows(base, d):
        return pl.ds(base + d, 8, stride=DH)

    tokens, zero = [[]], []

    def tie(val, kind):
        if kind & CFG["ties"]:
            tokens[-1].append(pltpu.bitcast(val, u32))

    def tied(rhs):
        tokens.append([])
        due = tokens.pop(0) if len(tokens) > CFG["lag"] else []
        if not due:
            return rhs
        words = pltpu.bitcast(rhs, u32)
        head = words[:8, :128] | (functools.reduce(jnp.bitwise_or, due) & zero[0])
        if words.shape[1] > 128:
            head = jnp.concatenate([head, words[:8, 128:]], axis=1)
        return pltpu.bitcast(jnp.concatenate([head, words[8:]], axis=0), bf16)

    wT, woT, xT, gate, oT = {}, {}, {}, {}, {}
    w_ready = set()

    def prep_qkv(p, g):
        base = p * D + g * GR
        for t in range(base // 128, (base + GR - 1) // 128 + 1):
            if t not in w_ready:
                w_ready.add(t)
                for c in range(NC):
                    tmp[c, lanes(t), :] = pltpu.bitcast(
                        wqkv_v[pl.ds(c * 64, 64), lanes(t)], bf16).astype(f32).T
                    yield 60
        parts = []
        for d in range(0, DH, 2):
            two = jnp.concatenate([load_rows(tmp, head_major_rows(base, d)),
                                   load_rows(tmp, head_major_rows(base, d + 1))], axis=0)
            parts.append(two.astype(bf16))
            yield 30
        wT[p, g] = jnp.concatenate(parts, axis=0)

    def prep_wo():
        for c in range(NC):
            perm = jnp.concatenate(
                [wo_v[c, pl.ds(g * GR // 2 + dp, 8, stride=DH // 2), :]
                 for g in range(HG) for dp in range(DH // 2)], axis=0)
            woT[c] = pltpu.bitcast(perm, bf16).T
            yield 200

    def prep_x(i):
        for u in range(NU):
            cols = []
            for c in range(NC):
                cols.append(pltpu.bitcast(x_v[c, slab(i, u), :], bf16).T)
                yield 40
            xT[i, u] = jnp.concatenate(cols, axis=0)

    def gates(i):
        gw = gw_ref[...].astype(f32).reshape(1, D)
        wr = wr_ref[...].astype(f32).reshape(1, D)
        for u in range(NU):
            g_acc = r_acc = None
            for c in range(NC):
                xs = pltpu.bitcast(x_v[c, slab(i, u), :], bf16).astype(f32)
                gp, rp = xs * gw[:, c * 128:(c + 1) * 128], xs * wr[:, c * 128:(c + 1) * 128]
                g_acc = gp if c == 0 else g_acc + gp
                r_acc = rp if c == 0 else r_acc + rp
                yield 80
            gt = jax.nn.sigmoid(jnp.sum(g_acc, axis=1, keepdims=True))
            gate[i, u] = jnp.broadcast_to(gt, (128, 128))
            tie(functools.reduce(jnp.add, [gate[i, u][r:r + 8] for r in range(0, 128, 8)]), 4)
            score_s[pl.ds(i * NU + u, 1), :] = jnp.sum(r_acc.T, axis=0, keepdims=True)
            yield 200

    lane = lax.broadcasted_iota(jnp.int32, (1, 128), 1)
    query, raw, logit, prob, inv, acc = {}, {}, {}, {}, {}, {}

    def taps(p, i, g, t, d, cur):
        prev = raw.pop((p, g, t, d)) if i > 0 else 0.0
        if i + 1 < NB:
            raw[p, g, t, d] = cur
        for wrap in range((W - 1 + NU - 1) // NU + 1):
            us = [u for u in range(NU) if 0 <= u - t + wrap * NU < W]
            if us:
                x = cur if wrap == 0 else pltpu.roll(
                    jnp.where(lane >= 128 - 2 * wrap, prev, cur), 2 * wrap, 1)
                for u in us:
                    yield u, u - t + wrap * NU, x

    def scores(i, g, t, k):
        for d in range(DH):
            for u, w, x in taps(1, i, g, t, d, k[d * 8:(d + 1) * 8]):
                term = query[i, g, u][d * 8:(d + 1) * 8] * x
                logit[u, w] = logit[u, w] + term if d else term

    def softmax(i, g):
        for u in range(NU):
            ls = []
            for w in range(W):
                l = logit.pop((u, w))
                if i == 0 and w > u:
                    l = jnp.where(lane >= 2 * ((w - u + NU - 1) // NU), l, MASKED)
                ls.append(l)
            m = functools.reduce(jnp.maximum, ls)
            for w in range(W):
                prob[u, w] = jnp.exp2((ls[w] - m) * EXP_SCALE)
            inv[u] = 1.0 / functools.reduce(jnp.add, [prob[u, w] for w in range(W)])

    def values(i, g, t, v):
        for d in range(DH):
            for u, w, x in taps(2, i, g, t, d, v[d * 8:(d + 1) * 8]):
                term = prob[u, w] * x
                acc[u, d] = acc[u, d] + term if (u, d) in acc else term
            if t == NU - 1 and d % 2:
                for u in range(NU):
                    pair = [acc.pop((u, d - 1)) * inv[u], acc.pop((u, d)) * inv[u]]
                    oT.setdefault((i, u), []).append(pltpu.bitcast(
                        pltpu.pack_elementwise(pair, packed_dtype=bf16), u32))

    def project(work, t):
        for i in sorted({i for _, i, _ in work}):
            mine = [(p, g) for p, ii, g in work if ii == i]
            r = jnp.dot(jnp.concatenate([wT[pg] for pg in mine], axis=0), tied(xT[i, t]),
                        preferred_element_type=f32)
            for n, (p, g) in enumerate(mine):
                part = r[n * GR:(n + 1) * GR]
                if p == 0:
                    query[i, g, t] = part
                else:
                    (scores, values)[p - 1](i, g, t, part)

    jobs, slow = [], []

    def background(budget, queue=jobs):
        while queue and budget > 0:
            cost = next(queue[0], None)
            if cost is None:
                queue.pop(0)
            else:
                budget -= cost

    picks = []

    def route():
        r = score_s[...]
        r = r.astype(bf16).astype(f32)
        key = jnp.where(r != r, -jnp.inf, r)
        sub = lax.broadcasted_iota(jnp.int32, (NB * NU, 128), 0)
        pos = (sub // NU) * TB + (lane // 2) * (2 * NU) + (sub % NU) * 2 + lane % 2
        free = pos >= 0
        for _ in range(2):
            m = jnp.max(jnp.where(free, key, -jnp.inf), keepdims=True)
            idx = jnp.min(jnp.where(free & (key == m), pos, S - 1))
            score = jnp.sum(jnp.where(pos == idx, r, 0.0), keepdims=True)
            free = free & (pos != idx)
            picks.append((idx, jax.nn.sigmoid(score)))
            yield 50

    row = lax.broadcasted_iota(jnp.int32, (16, D), 0)
    hidden = []

    def halves(ref, j):
        word = ref[pl.ds(8 * j, 8), :]
        return [pltpu.unpack_elementwise(word, index=n, packed_dtype=bf16, unpacked_dtype=f32)
                for n in range(2)]

    def picked(idx):
        tile = pl.ds(pl.multiple_of((idx // 16) * 8, 8), 8)
        return tile, row == idx % 16, load_bf16(x_v, tile).astype(f32)

    def ffn_hidden():
        xs = []
        for idx, _ in picks:
            _, hit, cur = picked(idx)
            xs.append(jnp.broadcast_to(
                jnp.sum(jnp.where(hit, cur, 0.0), axis=0, keepdims=True), (8, D)))

        def matvec(w, x):
            prod = w * x
            part = functools.reduce(
                jnp.add, [prod[:, c * 128:(c + 1) * 128] for c in range(NC)])
            return jnp.sum(part, axis=1, keepdims=True)

        for j in range(F // 16):
            hs = []
            for wg, wu in zip(halves(wg_v, j), halves(wu_v, j)):
                for x in xs:
                    half = 0.5 * matvec(wg, x)
                    h = (half * jnp.tanh(half) + half) * matvec(wu, x)
                    hs.append(jnp.broadcast_to(h, (8, 128)).astype(bf16).astype(f32))
            hidden.append(hs)
            tie(functools.reduce(jnp.add, hs), 1)
            yield 130

    def ffn_out():
        ys = [None] * len(picks)
        for j in range(F // 16):
            for n, wd in enumerate(halves(wd_v, j)):
                for k in range(len(picks)):
                    term = wd * jnp.tile(hidden[j][n * len(picks) + k], (1, NC))
                    ys[k] = term if ys[k] is None else ys[k] + term
            if j % 4 == 3:
                for y in ys:
                    for c in range(NC):
                        tie(y[:, c * 128:(c + 1) * 128], 2)
            yield 50
        for (idx, weight), y in zip(picks, ys):
            tile, hit, cur = picked(idx)
            y = jnp.sum(y, axis=0, keepdims=True) * weight
            store_bf16(x_v, tile, jnp.where(hit, cur + y, cur))

    def emit(i, cs):
        rhs = jnp.concatenate(
            [pltpu.bitcast(jnp.concatenate(oT[i, u], axis=0), bf16) for u in range(NU)], axis=1)
        aT = jnp.dot(jnp.concatenate([woT[c] for c in cs], axis=0), tied(rhs),
                     preferred_element_type=f32)
        for n, c in enumerate(cs):
            for u in range(NU):
                a = aT[n * 128:(n + 1) * 128, u * 128:(u + 1) * 128].T
                b = pltpu.bitcast(x_v[c, slab(i, u), :], bf16).astype(f32)
                gt = gate[i, u]
                o = gt * a + (1.0 - gt) * b
                out_v[c, slab(i, u), :] = pltpu.bitcast(o.astype(bf16), u32)
            cp_out(i, c).start()

    def scope(name):
        return jax.named_scope("@" + name) if CFG["scopes"] else contextlib.nullcontext()

    n_groups = NB * HG
    steps = [[(p, n // HG, n % HG) for p, n in CFG["order"](s) if 0 <= n < n_groups]
             for s in range(-1, n_groups + 1)]

    def w_tiles(work):
        return [t for p, i, g in work
                for t in range((p * D + g * GR) // 128, (p * D + g * GR + GR - 1) // 128 + 1)]

    seen = set()

    def w_batch(lo, hi):
        new = [t for work in steps[lo:hi] for t in w_tiles(work)]
        new = [t for t in dict.fromkeys(new) if t not in seen]
        seen.update(new)
        runs = [[t for _, t in run] for _, run in
                itertools.groupby(enumerate(sorted(new)), lambda nt: nt[1] - nt[0])]
        cols = [pl.ds(run[0] * 128, len(run) * 128) for run in runs]
        return [copy(wqkv_hbm.at[:, cl], wqkv_v.at[:, cl]) for cl in cols]

    batch = dict(w0=w_batch(0, 1), w1=w_batch(1, 2), w2=w_batch(2, 3), w3=w_batch(3, len(steps)),
                 x0=cp_x(0, 1), x1=cp_x(1, 2), x2=cp_x(2, NB),
                 wo=[copy(wo_hbm.at[:, lanes(c)], wo_v.at[c]) for c in range(NC)],
                 wg=[copy(wg_hbm, wg_v)], wu=[copy(wu_hbm, wu_v)], wd=[copy(wd_hbm, wd_v)])
    flying = []

    def run(actions):
        cost = 0
        for act, arg in actions:
            if act == "start":
                start(batch[arg])
                flying.append(arg)
            elif act == "wait":
                wait(batch[arg])
                flying.remove(arg)
            elif act == "w":
                for p, i, g in steps[arg]:
                    if i == 0:
                        jobs.append(prep_qkv(p, g))
                        cost += 700
            else:
                job, c = dict(x=(prep_x, 800), gates=(gates, 2400), wo=(prep_wo, 1000),
                              route=(route, 100), hidden=(ffn_hidden, 0), out=(ffn_out, 0))[act]
                (slow if act in ("hidden", "out") else jobs).append(job(*arg))
                cost += c
        return cost

    for actions in CFG["head"]:
        run(actions)
        background(1e9)
    zero.append((x_v[0, 0:8, :] >> 31) >> 1)
    for s, work in enumerate(steps):
        with scope(f"s{s}"):
            cost = 0
            for t in range(NU):
                cost += run(CFG["events"].get((s, t), ()))
                project(work, t)
                share = cost / (NU - t)
                background(share)
                cost -= share
                background(CFG["slow"].get(s, 0) / NU, slow)
            background(1e9)
            for p, i, g in work:
                if p == 1:
                    softmax(i, g)
        if s == CFG.get("stop"):
            out_v[0, 0:8, :] = pltpu.bitcast(functools.reduce(
                jnp.add, list(prob.values()) + list(inv.values()) + [v[:8] for v in query.values()]), u32)
            for ws in oT.values():
                for k, word in enumerate(ws):
                    out_v[1, pl.ds(8 * k, 8), :] = word
            wait([c for nm in flying for c in batch[nm]])
            cp_out(0, 0).start()
            cp_out(0, 0).wait()
            return
    background(1e9, slow)
    for i in range(NB):
        with scope(f"c{i}"):
            for cs in CFG["cs"]:
                emit(i, cs)
    wait([cp_out(i, c) for i in range(NB) for c in range(NC)])


@jax.jit
def pallas_gated_mix__sliding_local_dilated__moe_arch_mod__prompt_kernel(
    A_x: jax.Array,
    A_wqkv: jax.Array,
    A_wo: jax.Array,
    B_x: jax.Array,
    B_w_r: jax.Array,
    B_w_gate: jax.Array,
    B_w_up: jax.Array,
    B_w_down: jax.Array,
    gate_w: jax.Array,
):
    hbm = pl.BlockSpec(memory_space=pl.ANY)
    vmem = pl.BlockSpec(memory_space=pltpu.VMEM)
    return pl.pallas_call(
        _kernel,
        out_shape=jax.ShapeDtypeStruct((S, D), A_x.dtype),
        in_specs=[hbm, hbm, hbm, vmem, hbm, hbm, hbm, vmem],
        out_specs=hbm,
        interpret=CFG["interpret"],
        scratch_shapes=[
            pltpu.VMEM((NC, S // 2, 128), u32),
            pltpu.VMEM((D // 2, 3 * D), u32),
            pltpu.VMEM((NC, D // 2, 128), u32),
            pltpu.VMEM((F // 2, D), u32),
            pltpu.VMEM((F // 2, D), u32),
            pltpu.VMEM((F // 2, D), u32),
            pltpu.VMEM((NC, S // 2, 128), u32),
            pltpu.VMEM((NC, 3 * D, 128), f32),
            pltpu.VMEM((NB * NU, 128), f32),
            pltpu.SemaphoreType.DMA((64,)),
            pltpu.SemaphoreType.DMA((NB, NC)),
        ],
        compiler_params=pltpu.CompilerParams(
            vmem_limit_bytes=100 * 1024 * 1024, flags=CFG["flags"]),
    )(A_x.reshape(S, D), A_wqkv, A_wo, B_w_r, B_w_gate.T, B_w_up.T, B_w_down,
      gate_w).reshape(A_x.shape)
```

```python
import contextlib
import functools
import itertools
import math

import jax
import jax.numpy as jnp
from jax import lax
import jax.experimental.pallas as pl
import jax.experimental.pallas.tpu as pltpu

CFG = dict(
    flags=None, interpret=False, scopes=False,
    head=([("start", "w0"), ("start", "x0"), ("wait", "w0"), ("start", "w1"), ("w", 0)],
          [("wait", "x0"), ("start", "w2"), ("x", (0,))]),
    events={
        (0, 2): [("wait", "w1"), ("start", "w3"), ("w", 1)],
        (1, 1): [("wait", "w2"), ("start", "x1"), ("w", 2)],
        (2, 0): [("wait", "w3"), ("start", "x2"), ("w", 3)],
        (3, 0): [("wait", "x1"), ("w", 4), ("x", (1,))],
        (4, 0): [("wait", "x2"), ("start", "rest"), ("w", 5)],
        (5, 0): [("router", (0,))],
        (6, 0): [("router", (1,))],
        (7, 0): [("x", (2,)), ("router", (2,))],
        (8, 0): [("router", (3,))],
        (9, 0): [("route", ())],
        (10, 0): [("wait", "rest"), ("hidden", ()), ("out", ())],
        (11, 0): [("x", (3,))],
        (14, 0): [("wo", ())],
    },
    ties=0, lag=3,
    slow={10: 3200, 11: 2800, 12: 3200, 13: 3200, 14: 2800, 15: 3200, 16: 1200},
    hold=0, slow_c=800,
    order=lambda s: ((1, s), (2, s - 1), (0, s + 1)),
    cs=[(cs, (0, 1, 2, 3)) for cs in ((0, 1), (2, 3), (4,))],
    last=[((0, 1), (0, 1, 2, 3)), ((2, 3), (0, 1, 2, 3))] + [((4,), (u,)) for u in range(4)])

S, D, H, F = 2048, 640, 32, 1728
DH = D // H
W = 8
HG = H // 8
GR = 8 * DH
TB = 512
NB = S // TB
NU = TB // 128
NC = D // 128
NE = W - 1
N_SEMS = 9
SCALE = DH ** -0.5
EXP_SCALE = SCALE * math.log2(math.e)
MASKED = -1e9 / SCALE

f32, bf16, u32 = jnp.float32, jnp.bfloat16, jnp.uint32
NT = (((1,), (1,)), ((), ()))


def _kernel(x_hbm, wqkv_hbm, wo_hbm, wr_hbm, wg_hbm, wu_hbm, wd_hbm, gw_hbm,
            out_hbm,
            x_v, wqkv_v, wo_v, wg_v, wu_v, wd_v, out_v,
            tmp, score_s, wr_ref, gw_ref, sems):
    free_sems = iter(range(1, N_SEMS))

    def copies(pairs):
        sem = sems.at[next(free_sems)]
        return [pltpu.make_async_copy(src, dst, sem) for src, dst in pairs]

    def start(cps):
        for c in cps:
            c.start()

    def wait(cps):
        for c in cps:
            c.wait()

    def rows(i):
        return pl.ds(pl.multiple_of(i * (TB // 2), TB // 2), TB // 2)

    def lanes(c):
        return pl.ds(c * 128, 128)

    x_hbm, out_hbm, wqkv_hbm, wo_hbm, wg_hbm, wu_hbm, wd_hbm = (
        r.bitcast(u32) for r in (x_hbm, out_hbm, wqkv_hbm, wo_hbm, wg_hbm, wu_hbm, wd_hbm))

    def cp_x(lo, hi, extra=()):
        rws = pl.ds(lo * (TB // 2), (hi - lo) * (TB // 2))
        return copies([(x_hbm.at[rws, lanes(c)], x_v.at[c, rws]) for c in range(NC)] + list(extra))

    def cp_out(i, c):
        return pltpu.make_async_copy(out_v.at[c, rows(i)], out_hbm.at[rows(i), lanes(c)],
                                     sems.at[0])

    def slab(i, u):
        return pl.ds(i * (TB // 2) + u, 64, stride=NU)

    def load_rows(ref, rws=slice(None)):
        return jnp.concatenate([ref[c, rws, :] for c in range(ref.shape[0])], axis=1)

    def load_bf16(ref, rws=slice(None)):
        return pltpu.bitcast(load_rows(ref, rws), bf16)

    def store_bf16(ref, rws, val):
        val = pltpu.bitcast(val.astype(bf16), u32)
        for c in range(ref.shape[0]):
            ref[c, rws, :] = val[:, c * 128:(c + 1) * 128]

    def head_major_rows(base, d):
        return pl.ds(base + d, 8, stride=DH)

    wT, woT, xT, gate, oT = {}, {}, {}, {}, {}
    w_ready = set()

    def prep_qkv(p, g):
        base = p * D + g * GR
        for t in range(base // 128, (base + GR - 1) // 128 + 1):
            if t not in w_ready:
                w_ready.add(t)
                for c in range(NC):
                    tmp[c, lanes(t), :] = pltpu.bitcast(
                        wqkv_v[pl.ds(c * 64, 64), lanes(t)], bf16).astype(f32).T
                    yield 60
        parts = []
        for d in range(0, DH, 2):
            two = jnp.concatenate([load_rows(tmp, head_major_rows(base, d)),
                                   load_rows(tmp, head_major_rows(base, d + 1))], axis=0)
            parts.append(two.astype(bf16))
            yield 30
        wT[p, g] = jnp.concatenate(parts, axis=0)

    def prep_wo():
        for c in range(NC):
            perm = jnp.concatenate(
                [wo_v[c, pl.ds(g * GR // 2 + dp, 8, stride=DH // 2), :]
                 for g in range(HG) for dp in range(DH // 2)], axis=0)
            woT[c] = pltpu.bitcast(perm, bf16).T
            yield 200

    def prep_x(i):
        for u in range(NU):
            cols = []
            for c in range(NC):
                cols.append(pltpu.bitcast(x_v[c, slab(i, u), :], bf16).T)
                yield 40
            xT[i, u] = jnp.concatenate(cols, axis=0)

    def router(i):
        wr = wr_ref[...].astype(f32).reshape(1, D)
        for u in range(NU):
            acc_r = None
            for c in range(NC):
                xs = pltpu.bitcast(x_v[c, slab(i, u), :], bf16).astype(f32)
                term = xs * wr[:, c * 128:(c + 1) * 128]
                acc_r = term if c == 0 else acc_r + term
                yield 50
            score_s[pl.ds(i * NU + u, 1), :] = jnp.sum(acc_r.T, axis=0, keepdims=True)
            yield 50

    lane = lax.broadcasted_iota(jnp.int32, (1, 128), 1)
    query, raw, logit, prob, inv, acc = {}, {}, {}, {}, {}, {}

    def taps(p, i, g, t, d, cur):
        prev = raw.pop((p, g, t, d)) if i > 0 else 0.0
        if i + 1 < NB:
            raw[p, g, t, d] = cur
        for wrap in range((W - 1 + NU - 1) // NU + 1):
            us = [u for u in range(NU) if 0 <= u - t + wrap * NU < W]
            if us:
                x = cur if wrap == 0 else pltpu.roll(
                    jnp.where(lane >= 128 - 2 * wrap, prev, cur), 2 * wrap, 1)
                for u in us:
                    yield u, u - t + wrap * NU, x

    def scores(i, g, t, k):
        for d in range(DH):
            for u, w, x in taps(1, i, g, t, d, k[d * 8:(d + 1) * 8]):
                term = query[i, g, u][d * 8:(d + 1) * 8] * x
                logit[u, w] = logit[u, w] + term if d else term

    def softmax(i, g):
        for u in range(NU):
            ls = []
            for w in range(W):
                l = logit.pop((u, w))
                if i == 0 and w > u:
                    l = jnp.where(lane >= 2 * ((w - u + NU - 1) // NU), l, MASKED)
                ls.append(l)
            m = functools.reduce(jnp.maximum, ls)
            for w in range(W):
                prob[u, w] = jnp.exp2((ls[w] - m) * EXP_SCALE)
            inv[u] = 1.0 / functools.reduce(jnp.add, [prob[u, w] for w in range(W)])

    def values(i, g, t, v):
        for d in range(DH):
            for u, w, x in taps(2, i, g, t, d, v[d * 8:(d + 1) * 8]):
                term = prob[u, w] * x
                acc[u, d] = acc[u, d] + term if (u, d) in acc else term
            if t == NU - 1 and d % 2:
                for u in range(NU):
                    pair = [acc.pop((u, d - 1)) * inv[u], acc.pop((u, d)) * inv[u]]
                    oT.setdefault((i, u), []).append(pltpu.bitcast(
                        pltpu.pack_elementwise(pair, packed_dtype=bf16), u32))

    def project(work, t):
        for i in sorted({i for _, i, _ in work}):
            mine = [(p, g) for p, ii, g in work if ii == i]
            lhs = [wT[pg] for pg in mine]
            if (0, 0) in mine:
                gw = gw_ref[...].astype(f32).reshape(1, D)
                lhs.append(jnp.broadcast_to(gw, (16, D)).astype(bf16))
            r = jnp.dot(jnp.concatenate(lhs, axis=0), xT[i, t], preferred_element_type=f32)
            if (0, 0) in mine:
                gt = jax.nn.sigmoid(r[len(mine) * GR:len(mine) * GR + 8])
                gate[i, t] = jnp.tile(gt, (16, 1)).T
            for n, (p, g) in enumerate(mine):
                part = r[n * GR:(n + 1) * GR]
                if p == 0:
                    query[i, g, t] = part
                else:
                    (scores, values)[p - 1](i, g, t, part)

    jobs, slow = [], []

    def background(budget, queue=jobs):
        while queue and budget > 0:
            cost = next(queue[0], None)
            if cost is None:
                queue.pop(0)
            else:
                budget -= cost

    picks = []

    def route():
        r = score_s[...]
        r = r.astype(bf16).astype(f32)
        key = jnp.where(r != r, -jnp.inf, r)
        sub = lax.broadcasted_iota(jnp.int32, (NB * NU, 128), 0)
        pos = (sub // NU) * TB + (lane // 2) * (2 * NU) + (sub % NU) * 2 + lane % 2
        free = pos >= 0
        for _ in range(2):
            m = jnp.max(jnp.where(free, key, -jnp.inf), keepdims=True)
            idx = jnp.min(jnp.where(free & (key == m), pos, S - 1))
            score = jnp.sum(jnp.where(pos == idx, r, 0.0), keepdims=True)
            free = free & (pos != idx)
            picks.append((idx, jax.nn.sigmoid(score)))
            yield 50

    row = lax.broadcasted_iota(jnp.int32, (16, D), 0)
    hidden = []

    def halves(ref, j):
        word = ref[pl.ds(8 * j, 8), :]
        return [pltpu.unpack_elementwise(word, index=n, packed_dtype=bf16, unpacked_dtype=f32)
                for n in range(2)]

    def picked(idx):
        tile = pl.ds(pl.multiple_of((idx // 16) * 8, 8), 8)
        return tile, row == idx % 16, load_bf16(x_v, tile).astype(f32)

    def ffn_hidden():
        xs = []
        for idx, _ in picks:
            _, hit, cur = picked(idx)
            xs.append(jnp.broadcast_to(
                jnp.sum(jnp.where(hit, cur, 0.0), axis=0, keepdims=True), (8, D)))

        def matvec(w, x):
            prod = w * x
            part = functools.reduce(
                jnp.add, [prod[:, c * 128:(c + 1) * 128] for c in range(NC)])
            return jnp.sum(part, axis=1, keepdims=True)

        for j in range(F // 16):
            hs = []
            for wg, wu in zip(halves(wg_v, j), halves(wu_v, j)):
                for x in xs:
                    half = 0.5 * matvec(wg, x)
                    h = (half * jnp.tanh(half) + half) * matvec(wu, x)
                    hs.append(jnp.broadcast_to(h, (8, 128)).astype(bf16).astype(f32))
            hidden.append(hs)
            yield 130

    def ffn_out():
        ys = [None] * len(picks)
        for j in range(F // 16):
            for n, wd in enumerate(halves(wd_v, j)):
                for k in range(len(picks)):
                    term = wd * jnp.tile(hidden[j][n * len(picks) + k], (1, NC))
                    ys[k] = term if ys[k] is None else ys[k] + term
            yield 50
        for (idx, weight), y in zip(picks, ys):
            tile, hit, cur = picked(idx)
            y = jnp.sum(y, axis=0, keepdims=True) * weight
            store_bf16(x_v, tile, jnp.where(hit, cur + y, cur))

    def out_proj(i, cs, us):
        rhs = jnp.concatenate(
            [pltpu.bitcast(jnp.concatenate(oT[i, u], axis=0), bf16) for u in us], axis=1)
        aT = jnp.dot(jnp.concatenate([woT[c] for c in cs], axis=0), rhs,
                     preferred_element_type=f32)
        return {(c, u): aT[n * 128:(n + 1) * 128, m * 128:(m + 1) * 128]
                for n, c in enumerate(cs) for m, u in enumerate(us)}

    def mix(i, tiles):
        for (c, u), aT in tiles.items():
            b = pltpu.bitcast(x_v[c, slab(i, u), :], bf16).astype(f32)
            o = gate[i, u] * aT.T + (1.0 - gate[i, u]) * b
            out_v[c, slab(i, u), :] = pltpu.bitcast(o.astype(bf16), u32)
            if u == NU - 1:
                cp_out(i, c).start()

    def scope(name):
        return jax.named_scope("@" + name) if CFG["scopes"] else contextlib.nullcontext()

    n_groups = NB * HG
    steps = [[(p, n // HG, n % HG) for p, n in CFG["order"](s) if 0 <= n < n_groups]
             for s in range(-1, n_groups + 1)]

    def w_tiles(work):
        return [t for p, i, g in work
                for t in range((p * D + g * GR) // 128, (p * D + g * GR + GR - 1) // 128 + 1)]

    seen = set()

    def w_batch(lo, hi):
        new = [t for work in steps[lo:hi] for t in w_tiles(work)]
        new = [t for t in dict.fromkeys(new) if t not in seen]
        seen.update(new)
        runs = [[t for _, t in run] for _, run in
                itertools.groupby(enumerate(sorted(new)), lambda nt: nt[1] - nt[0])]
        cols = [pl.ds(run[0] * 128, len(run) * 128) for run in runs]
        return copies((wqkv_hbm.at[:, cl], wqkv_v.at[:, cl]) for cl in cols)

    batch = dict(w0=w_batch(0, 1), w1=w_batch(1, 2), w2=w_batch(2, 3), w3=w_batch(3, len(steps)),
                 x0=cp_x(0, 1, [(gw_hbm, gw_ref), (wr_hbm, wr_ref)]), x1=cp_x(1, 2), x2=cp_x(2, NB),
                 rest=copies([(wg_hbm, wg_v), (wu_hbm, wu_v), (wd_hbm, wd_v)] +
                             [(wo_hbm.at[:, lanes(c)], wo_v.at[c]) for c in range(NC)]))
    flying = []

    def run(actions):
        cost = 0
        for act, arg in actions:
            if act == "start":
                start(batch[arg])
                flying.append(arg)
            elif act == "wait":
                with scope(arg):
                    wait(batch[arg])
                flying.remove(arg)
            elif act == "w":
                for p, i, g in steps[arg]:
                    if i == 0:
                        jobs.append(prep_qkv(p, g))
                        cost += 700
            else:
                job, c = dict(x=(prep_x, 800), router=(router, 1200), wo=(prep_wo, 1000),
                              route=(route, 100), hidden=(ffn_hidden, 0), out=(ffn_out, 0))[act]
                (slow if act in ("hidden", "out") else jobs).append(job(*arg))
                cost += c
        return cost

    for actions in CFG["head"]:
        run(actions)
        background(1e9)
    for s, work in enumerate(steps):
        with contextlib.nullcontext():
            cost = 0
            for t in range(NU):
                cost += run(CFG["events"].get((s, t), ()))
                project(work, t)
                share = cost / (NU - t)
                background(share)
                cost -= share
                background(CFG["slow"].get(s, 0) / NU, slow)
            background(1e9)
            for p, i, g in work:
                if p == 1:
                    softmax(i, g)
        if s == CFG.get("stop"):
            out_v[0, 0:8, :] = pltpu.bitcast(functools.reduce(
                jnp.add, list(prob.values()) + list(inv.values()) + [v[:8] for v in query.values()]), u32)
            for ws in oT.values():
                for k, word in enumerate(ws):
                    out_v[1, pl.ds(8 * k, 8), :] = word
            wait([c for nm in flying for c in batch[nm]])
            cp_out(0, 0).start()
            cp_out(0, 0).wait()
            return
    pieces = [(i, cs, us) for i in range(NB)
              for cs, us in CFG["last" if i == NB - 1 else "cs"]]
    held = []
    for n, (i, cs, us) in enumerate(pieces):
        held.append((i, out_proj(i, cs, us)))
        if n < CFG["hold"]:
            background(CFG["slow_c"] * len(cs), slow)
            continue
        background(1e9, slow)
        for _ in range(2):
            if held:
                mix(*held.pop(0))
    for piece in held:
        mix(*piece)
    with scope("out"):
        wait([cp_out(i, c) for i in range(NB) for c in range(NC)])


@jax.jit
def pallas_gated_mix__sliding_local_dilated__moe_arch_mod__prompt_kernel(
    A_x: jax.Array,
    A_wqkv: jax.Array,
    A_wo: jax.Array,
    B_x: jax.Array,
    B_w_r: jax.Array,
    B_w_gate: jax.Array,
    B_w_up: jax.Array,
    B_w_down: jax.Array,
    gate_w: jax.Array,
):
    hbm = pl.BlockSpec(memory_space=pl.ANY)
    return pl.pallas_call(
        _kernel,
        out_shape=jax.ShapeDtypeStruct((S, D), A_x.dtype),
        in_specs=[hbm] * 8,
        out_specs=hbm,
        interpret=CFG["interpret"],
        scratch_shapes=[
            pltpu.VMEM((NC, S // 2, 128), u32),
            pltpu.VMEM((D // 2, 3 * D), u32),
            pltpu.VMEM((NC, D // 2, 128), u32),
            pltpu.VMEM((F // 2, D), u32),
            pltpu.VMEM((F // 2, D), u32),
            pltpu.VMEM((F // 2, D), u32),
            pltpu.VMEM((NC, S // 2, 128), u32),
            pltpu.VMEM((NC, 3 * D, 128), f32),
            pltpu.VMEM((NB * NU, 128), f32),
            pltpu.VMEM((D,), bf16),
            pltpu.VMEM((D,), bf16),
            pltpu.SemaphoreType.DMA((N_SEMS,)),
        ],
        compiler_params=pltpu.CompilerParams(
            vmem_limit_bytes=100 * 1024 * 1024, flags=CFG["flags"]),
    )(A_x.reshape(S, D), A_wqkv, A_wo, B_w_r, B_w_gate.T, B_w_up.T, B_w_down,
      gate_w).reshape(A_x.shape)
```

```python
import contextlib
import functools
import itertools
import math

import jax
import jax.numpy as jnp
from jax import lax
import jax.experimental.pallas as pl
import jax.experimental.pallas.tpu as pltpu

CFG = dict(
    flags=None, interpret=False, scopes=False,
    head=([("start", "w0"), ("start", "x0"), ("wait", "w0"), ("start", "w1"), ("w", 0)],
          [("wait", "x0"), ("start", "w2"), ("x", (0,))]),
    events={
        (0, 2): [("wait", "w1"), ("start", "w3"), ("w", 1)],
        (1, 1): [("wait", "w2"), ("start", "x1"), ("w", 2)],
        (2, 0): [("wait", "w3"), ("start", "x2"), ("w", 3)],
        (3, 0): [("wait", "x1"), ("w", 4), ("x", (1,))],
        (4, 0): [("wait", "x2"), ("start", "gu"), ("start", "rest"), ("w", 5)],
        (5, 0): [("router", (0,))],
        (6, 0): [("router", (1,))],
        (7, 0): [("x", (2,)), ("router", (2,))],
        (8, 0): [("router", (3,))],
        (9, 0): [("route", ())],
        (10, 0): [("wait", "gu"), ("wait", "rest"), ("hidden", ()), ("out", ())],
        (11, 0): [("x", (3,))],
        (14, 0): [("wo", ())],
    },
    ties=0, lag=3,
    slow={10: 3200, 11: 2800, 12: 3200, 13: 3200, 14: 2800, 15: 3200, 16: 1200},
    hold=0, bulk=True, w3=4, slow_c=800,
    order=lambda s: ((1, s), (2, s - 1), (0, s + 1)),
    cs=[((0, 1, 2, 3, 4), (0, 1)), ((0, 1, 2, 3, 4), (2, 3))],
    last=[((0, 1), (0, 1, 2, 3)), ((2, 3), (0, 1, 2, 3))] + [((4,), (u,)) for u in range(4)])

S, D, H, F = 2048, 640, 32, 1728
DH = D // H
W = 8
HG = H // 8
GR = 8 * DH
TB = 512
NB = S // TB
NU = TB // 128
NC = D // 128
NE = W - 1
N_SEMS = 10
SCALE = DH ** -0.5
EXP_SCALE = SCALE * math.log2(math.e)
MASKED = -1e9 / SCALE

f32, bf16, u32 = jnp.float32, jnp.bfloat16, jnp.uint32
NT = (((1,), (1,)), ((), ()))


def _kernel(x_hbm, wqkv_hbm, wo_hbm, wr_hbm, wg_hbm, wu_hbm, wd_hbm, gw_hbm,
            out_hbm,
            x_v, wqkv_v, wo_v, wg_v, wu_v, wd_v, out_v,
            tmp, score_s, wr_ref, gw_ref, sems):
    free_sems = iter(range(1, N_SEMS))

    def copies(pairs):
        sem = sems.at[next(free_sems)]
        return [pltpu.make_async_copy(src, dst, sem) for src, dst in pairs]

    def start(cps):
        for c in cps:
            c.start()

    def wait(cps):
        for c in cps:
            c.wait()

    def rows(i):
        return pl.ds(pl.multiple_of(i * (TB // 2), TB // 2), TB // 2)

    def lanes(c):
        return pl.ds(c * 128, 128)

    x_hbm, out_hbm, wqkv_hbm, wo_hbm, wg_hbm, wu_hbm, wd_hbm = (
        r.bitcast(u32) for r in (x_hbm, out_hbm, wqkv_hbm, wo_hbm, wg_hbm, wu_hbm, wd_hbm))

    def cp_x(lo, hi, extra=()):
        rws = pl.ds(lo * (TB // 2), (hi - lo) * (TB // 2))
        return copies([(x_hbm.at[rws, lanes(c)], x_v.at[c, rws]) for c in range(NC)] + list(extra))

    def cp_out(i, c):
        return pltpu.make_async_copy(out_v.at[c, rows(i)], out_hbm.at[rows(i), lanes(c)],
                                     sems.at[0])

    def slab(i, u):
        return pl.ds(i * (TB // 2) + u, 64, stride=NU)

    def load_rows(ref, rws=slice(None)):
        return jnp.concatenate([ref[c, rws, :] for c in range(ref.shape[0])], axis=1)

    def load_bf16(ref, rws=slice(None)):
        return pltpu.bitcast(load_rows(ref, rws), bf16)

    def store_bf16(ref, rws, val):
        val = pltpu.bitcast(val.astype(bf16), u32)
        for c in range(ref.shape[0]):
            ref[c, rws, :] = val[:, c * 128:(c + 1) * 128]

    def head_major_rows(base, d):
        return pl.ds(base + d, 8, stride=DH)

    wT, woT, xT, gate, oT = {}, {}, {}, {}, {}
    w_ready = set()

    def prep_qkv(p, g):
        base = p * D + g * GR
        for t in range(base // 128, (base + GR - 1) // 128 + 1):
            if t not in w_ready:
                w_ready.add(t)
                for c in range(NC):
                    tmp[c, lanes(t), :] = pltpu.bitcast(
                        wqkv_v[pl.ds(c * 64, 64), lanes(t)], bf16).astype(f32).T
                    yield 60
        parts = []
        for d in range(0, DH, 2):
            two = jnp.concatenate([load_rows(tmp, head_major_rows(base, d)),
                                   load_rows(tmp, head_major_rows(base, d + 1))], axis=0)
            parts.append(two.astype(bf16))
            yield 30
        wT[p, g] = jnp.concatenate(parts, axis=0)

    def prep_wo():
        for c in range(NC):
            perm = jnp.concatenate(
                [wo_v[c, pl.ds(g * GR // 2 + dp, 8, stride=DH // 2), :]
                 for g in range(HG) for dp in range(DH // 2)], axis=0)
            woT[c] = pltpu.bitcast(perm, bf16).T
            yield 200

    def prep_x(i):
        for u in range(NU):
            cols = []
            for c in range(NC):
                cols.append(pltpu.bitcast(x_v[c, slab(i, u), :], bf16).T)
                yield 40
            xT[i, u] = jnp.concatenate(cols, axis=0)

    def router(i):
        wr = wr_ref[...].astype(f32).reshape(1, D)
        for u in range(NU):
            acc_r = None
            for c in range(NC):
                xs = pltpu.bitcast(x_v[c, slab(i, u), :], bf16).astype(f32)
                term = xs * wr[:, c * 128:(c + 1) * 128]
                acc_r = term if c == 0 else acc_r + term
                yield 50
            score_s[pl.ds(i * NU + u, 1), :] = jnp.sum(acc_r.T, axis=0, keepdims=True)
            yield 50

    lane = lax.broadcasted_iota(jnp.int32, (1, 128), 1)
    query, raw, logit, prob, inv, acc = {}, {}, {}, {}, {}, {}

    def taps(p, i, g, t, d, cur):
        prev = raw.pop((p, g, t, d)) if i > 0 else 0.0
        if i + 1 < NB:
            raw[p, g, t, d] = cur
        for wrap in range((W - 1 + NU - 1) // NU + 1):
            us = [u for u in range(NU) if 0 <= u - t + wrap * NU < W]
            if us:
                x = cur if wrap == 0 else pltpu.roll(
                    jnp.where(lane >= 128 - 2 * wrap, prev, cur), 2 * wrap, 1)
                for u in us:
                    yield u, u - t + wrap * NU, x

    def scores(i, g, t, k):
        for d in range(DH):
            for u, w, x in taps(1, i, g, t, d, k[d * 8:(d + 1) * 8]):
                term = query[i, g, u][d * 8:(d + 1) * 8] * x
                logit[u, w] = logit[u, w] + term if d else term

    def softmax(i, g):
        for u in range(NU):
            ls = []
            for w in range(W):
                l = logit.pop((u, w))
                if i == 0 and w > u:
                    l = jnp.where(lane >= 2 * ((w - u + NU - 1) // NU), l, MASKED)
                ls.append(l)
            m = functools.reduce(jnp.maximum, ls)
            for w in range(W):
                prob[u, w] = jnp.exp2((ls[w] - m) * EXP_SCALE)
            inv[u] = 1.0 / functools.reduce(jnp.add, [prob[u, w] for w in range(W)])

    def values(i, g, t, v):
        for d in range(DH):
            for u, w, x in taps(2, i, g, t, d, v[d * 8:(d + 1) * 8]):
                term = prob[u, w] * x
                acc[u, d] = acc[u, d] + term if (u, d) in acc else term
            if t == NU - 1 and d % 2:
                for u in range(NU):
                    pair = [acc.pop((u, d - 1)) * inv[u], acc.pop((u, d)) * inv[u]]
                    oT.setdefault((i, u), []).append(pltpu.bitcast(
                        pltpu.pack_elementwise(pair, packed_dtype=bf16), u32))

    def project(work, t):
        results = []
        for i in sorted({i for _, i, _ in work}):
            mine = [(p, g) for p, ii, g in work if ii == i]
            lhs = [wT[pg] for pg in mine]
            if (0, 0) in mine:
                gw = gw_ref[...].astype(f32).reshape(1, D)
                lhs.append(jnp.broadcast_to(gw, (16, D)).astype(bf16))
            r = jnp.dot(jnp.concatenate(lhs, axis=0), xT[i, t], preferred_element_type=f32)
            results.append((i, mine, r))
        return results

    def consume(results, t):
        for i, mine, r in results:
            if (0, 0) in mine:
                gt = jax.nn.sigmoid(r[len(mine) * GR:len(mine) * GR + 8])
                gate[i, t] = jnp.tile(gt, (16, 1)).T
            for n, (p, g) in enumerate(mine):
                part = r[n * GR:(n + 1) * GR]
                if p == 0:
                    query[i, g, t] = part
                else:
                    (scores, values)[p - 1](i, g, t, part)

    jobs, slow = [], []

    def background(budget, queue=jobs):
        while queue and budget > 0:
            cost = next(queue[0], None)
            if cost is None:
                queue.pop(0)
            else:
                budget -= cost

    picks = []

    def route():
        r = score_s[...]
        r = r.astype(bf16).astype(f32)
        key = jnp.where(r != r, -jnp.inf, r)
        sub = lax.broadcasted_iota(jnp.int32, (NB * NU, 128), 0)
        pos = (sub // NU) * TB + (lane // 2) * (2 * NU) + (sub % NU) * 2 + lane % 2
        free = pos >= 0
        for _ in range(2):
            m = jnp.max(jnp.where(free, key, -jnp.inf), keepdims=True)
            idx = jnp.min(jnp.where(free & (key == m), pos, S - 1))
            score = jnp.sum(jnp.where(pos == idx, r, 0.0), keepdims=True)
            free = free & (pos != idx)
            picks.append((idx, jax.nn.sigmoid(score)))
            yield 50

    row = lax.broadcasted_iota(jnp.int32, (16, D), 0)
    hidden = []

    def halves(ref, j):
        word = ref[pl.ds(8 * j, 8), :]
        return [pltpu.unpack_elementwise(word, index=n, packed_dtype=bf16, unpacked_dtype=f32)
                for n in range(2)]

    def picked(idx):
        tile = pl.ds(pl.multiple_of((idx // 16) * 8, 8), 8)
        return tile, row == idx % 16, load_bf16(x_v, tile).astype(f32)

    def ffn_hidden():
        xs = []
        for idx, _ in picks:
            _, hit, cur = picked(idx)
            xs.append(jnp.broadcast_to(
                jnp.sum(jnp.where(hit, cur, 0.0), axis=0, keepdims=True), (8, D)))

        def matvec(w, x):
            prod = w * x
            part = functools.reduce(
                jnp.add, [prod[:, c * 128:(c + 1) * 128] for c in range(NC)])
            return jnp.sum(part, axis=1, keepdims=True)

        for j in range(F // 16):
            hs = []
            for wg, wu in zip(halves(wg_v, j), halves(wu_v, j)):
                for x in xs:
                    half = 0.5 * matvec(wg, x)
                    h = (half * jnp.tanh(half) + half) * matvec(wu, x)
                    hs.append(jnp.broadcast_to(h, (8, 128)))
            hidden.append(hs)
            yield 130

    def ffn_out():
        ys = [None] * len(picks)
        for j in range(F // 16):
            for n, wd in enumerate(halves(wd_v, j)):
                for k in range(len(picks)):
                    term = wd * jnp.tile(hidden[j][n * len(picks) + k], (1, NC))
                    ys[k] = term if ys[k] is None else ys[k] + term
            yield 50
        for (idx, weight), y in zip(picks, ys):
            tile, hit, cur = picked(idx)
            y = jnp.sum(y, axis=0, keepdims=True) * weight
            store_bf16(x_v, tile, jnp.where(hit, cur + y, cur))

    def out_proj(i, cs, us):
        rhs = jnp.concatenate(
            [pltpu.bitcast(jnp.concatenate(oT[i, u], axis=0), bf16) for u in us], axis=1)
        aT = jnp.dot(jnp.concatenate([woT[c] for c in cs], axis=0), rhs,
                     preferred_element_type=f32)
        return {(c, u): aT[n * 128:(n + 1) * 128, m * 128:(m + 1) * 128]
                for n, c in enumerate(cs) for m, u in enumerate(us)}

    def mix(i, tiles):
        for (c, u), aT in tiles.items():
            b = pltpu.bitcast(x_v[c, slab(i, u), :], bf16).astype(f32)
            o = gate[i, u] * aT.T + (1.0 - gate[i, u]) * b
            out_v[c, slab(i, u), :] = pltpu.bitcast(o.astype(bf16), u32)
            if u == NU - 1 and (i == NB - 1 or not CFG["bulk"]):
                cp_out(i, c).start()
            elif (u, c) == (NU - 1, NC - 1):
                start([cp_out(i, n) for n in range(NC)])

    def scope(name):
        return jax.named_scope("@" + name) if CFG["scopes"] else contextlib.nullcontext()

    n_groups = NB * HG
    steps = [[(p, n // HG, n % HG) for p, n in CFG["order"](s) if 0 <= n < n_groups]
             for s in range(-1, n_groups + 1)]

    def w_tiles(work):
        return [t for p, i, g in work
                for t in range((p * D + g * GR) // 128, (p * D + g * GR + GR - 1) // 128 + 1)]

    seen = set()

    def w_pairs(lo, hi):
        new = [t for work in steps[lo:hi] for t in w_tiles(work)]
        new = [t for t in dict.fromkeys(new) if t not in seen]
        seen.update(new)
        runs = [[t for _, t in run] for _, run in
                itertools.groupby(enumerate(sorted(new)), lambda nt: nt[1] - nt[0])]
        cols = [pl.ds(run[0] * 128, len(run) * 128) for run in runs]
        return [(wqkv_hbm.at[:, cl], wqkv_v.at[:, cl]) for cl in cols]

    batch = dict(w0=copies(w_pairs(0, 1)), w1=copies(w_pairs(1, 2)), w2=copies(w_pairs(2, 3)),
                 w3=copies(w_pairs(3, CFG["w3"])),
                 x0=cp_x(0, 1, [(gw_hbm, gw_ref), (wr_hbm, wr_ref)]), x1=cp_x(1, 2, w_pairs(3, len(steps))), x2=cp_x(2, NB),
                 gu=copies([(wg_hbm, wg_v), (wu_hbm, wu_v)]),
                 rest=copies([(wd_hbm, wd_v)] +
                             [(wo_hbm.at[:, lanes(c)], wo_v.at[c]) for c in range(NC)]))
    flying = []

    def run(actions):
        cost = 0
        for act, arg in actions:
            if act == "start":
                start(batch[arg])
                flying.append(arg)
            elif act == "wait":
                with scope(arg):
                    wait(batch[arg])
                flying.remove(arg)
            elif act == "w":
                for p, i, g in steps[arg]:
                    if i == 0:
                        jobs.append(prep_qkv(p, g))
                        cost += 700
            else:
                job, c = dict(x=(prep_x, 800), router=(router, 1200), wo=(prep_wo, 1000),
                              route=(route, 100), hidden=(ffn_hidden, 0), out=(ffn_out, 0))[act]
                (slow if act in ("hidden", "out") else jobs).append(job(*arg))
                cost += c
        return cost

    for actions in CFG["head"]:
        run(actions)
        background(1e9)
    for s, work in enumerate(steps):
        with contextlib.nullcontext():
            cost = 0
            for t in range(NU):
                cost += run(CFG["events"].get((s, t), ()))
                results = project(work, t)
                cost += run(CFG["events"].get((s, t + 0.5), ()))
                consume(results, t)
                share = cost / (NU - t)
                background(share)
                cost -= share
                background(CFG["slow"].get(s, 0) / NU, slow)
            background(1e9)
            for p, i, g in work:
                if p == 1:
                    softmax(i, g)
        if s == CFG.get("stop"):
            out_v[0, 0:8, :] = pltpu.bitcast(functools.reduce(
                jnp.add, list(prob.values()) + list(inv.values()) + [v[:8] for v in query.values()]), u32)
            for ws in oT.values():
                for k, word in enumerate(ws):
                    out_v[1, pl.ds(8 * k, 8), :] = word
            wait([c for nm in flying for c in batch[nm]])
            cp_out(0, 0).start()
            cp_out(0, 0).wait()
            return
    pieces = [(i, cs, us) for i in range(NB)
              for cs, us in CFG["last" if i == NB - 1 else "cs"]]
    held = []
    for n, (i, cs, us) in enumerate(pieces):
        held.append((i, out_proj(i, cs, us)))
        if n < CFG["hold"]:
            background(CFG["slow_c"] * len(cs), slow)
            continue
        background(1e9, slow)
        for _ in range(2):
            if held:
                mix(*held.pop(0))
    for piece in held:
        mix(*piece)
    with scope("out"):
        wait([cp_out(i, c) for i in range(NB) for c in range(NC)])


@jax.jit
def pallas_gated_mix__sliding_local_dilated__moe_arch_mod__prompt_kernel(
    A_x: jax.Array,
    A_wqkv: jax.Array,
    A_wo: jax.Array,
    B_x: jax.Array,
    B_w_r: jax.Array,
    B_w_gate: jax.Array,
    B_w_up: jax.Array,
    B_w_down: jax.Array,
    gate_w: jax.Array,
):
    hbm = pl.BlockSpec(memory_space=pl.ANY)
    return pl.pallas_call(
        _kernel,
        out_shape=jax.ShapeDtypeStruct((S, D), A_x.dtype),
        in_specs=[hbm] * 8,
        out_specs=hbm,
        interpret=CFG["interpret"],
        scratch_shapes=[
            pltpu.VMEM((NC, S // 2, 128), u32),
            pltpu.VMEM((D // 2, 3 * D), u32),
            pltpu.VMEM((NC, D // 2, 128), u32),
            pltpu.VMEM((F // 2, D), u32),
            pltpu.VMEM((F // 2, D), u32),
            pltpu.VMEM((F // 2, D), u32),
            pltpu.VMEM((NC, S // 2, 128), u32),
            pltpu.VMEM((NC, 3 * D, 128), f32),
            pltpu.VMEM((NB * NU, 128), f32),
            pltpu.VMEM((D,), bf16),
            pltpu.VMEM((D,), bf16),
            pltpu.SemaphoreType.DMA((N_SEMS,)),
        ],
        compiler_params=pltpu.CompilerParams(
            vmem_limit_bytes=100 * 1024 * 1024, flags=CFG["flags"]),
    )(A_x.reshape(S, D), A_wqkv, A_wo, B_w_r, B_w_gate.T, B_w_up.T, B_w_down,
      gate_w).reshape(A_x.shape)
```

```python
import contextlib
import functools
import itertools
import math

import jax
import jax.numpy as jnp
from jax import lax
import jax.experimental.pallas as pl
import jax.experimental.pallas.tpu as pltpu

CFG = dict(
    flags=None, interpret=False, scopes=False,
    head=(([("start", "w0"), ("start", "x0"), ("wait", "w0"), ("start", "w1"), ("w", 0)], 1e9),
          ([("wait", "x0"), ("start", "w2"), ("x", (0,))], 201)),
    nu=1, nu_from=5,
    events={
        (0, 2): [("wait", "w1"), ("start", "w3"), ("w", 1)],
        (1, 1): [("wait", "w2"), ("start", "x1"), ("w", 2)],
        (2, 0): [("wait", "w3"), ("start", "x2"), ("w", 3)],
        (3, 0): [("wait", "x1"), ("w", 4), ("x", (1,))],
        (4, 0): [("wait", "x2"), ("start", "gu"), ("start", "rest"), ("w", 5)],
        (5, 0): [("router", (0,)), ("router", (1,))],
        (6, 0): [("router", (2,))],
        (7, 0): [("x", (2,))],
        (8, 0): [("router", (3,))],
        (9, 0): [("route", ())],
        (10, 0): [("wait", "gu"), ("wait", "rest"), ("hidden", ()), ("out", ())],
        (11, 0): [("x", (3,))],
        (14, 0): [("wo", ())],
    },
    ties=0, lag=3,
    slow={10: 3600, 11: 3200, 12: 3600, 13: 3600, 14: 3200, 15: 3000},
    hold=0, bulk=True, w3=4, slow_c=800,
    order=lambda s: ((1, s), (2, s - 1), (0, s + 1)),
    cs=[((0, 1, 2, 3, 4), (0, 1)), ((0, 1, 2, 3, 4), (2, 3))],
    last=[((0, 1, 2), (0, 1)), ((0, 1, 2), (2, 3)), ((3,), (0, 1, 2, 3)),
          ((4,), (0, 1)), ((4,), (2,)), ((4,), (3,))])

S, D, H, F = 2048, 640, 32, 1728
DH = D // H
W = 8
HG = H // 8
GR = 8 * DH
TB = 512
NB = S // TB
NU = TB // 128
NC = D // 128
NE = W - 1
N_SEMS = 10
SCALE = DH ** -0.5
EXP_SCALE = SCALE * math.log2(math.e)
MASKED = -1e9 / SCALE

f32, bf16, u32 = jnp.float32, jnp.bfloat16, jnp.uint32
NT = (((1,), (1,)), ((), ()))


def _kernel(x_hbm, wqkv_hbm, wo_hbm, wr_hbm, wg_hbm, wu_hbm, wd_hbm, gw_hbm,
            out_hbm,
            x_v, wqkv_v, wo_v, wg_v, wu_v, wd_v, out_v,
            tmp, score_s, wr_ref, gw_ref, sems):
    free_sems = iter(range(1, N_SEMS))

    def copies(pairs):
        sem = sems.at[next(free_sems)]
        return [pltpu.make_async_copy(src, dst, sem) for src, dst in pairs]

    def start(cps):
        for c in cps:
            c.start()

    def wait(cps):
        for c in cps:
            c.wait()

    def rows(i):
        return pl.ds(pl.multiple_of(i * (TB // 2), TB // 2), TB // 2)

    def lanes(c):
        return pl.ds(c * 128, 128)

    x_hbm, out_hbm, wqkv_hbm, wo_hbm, wg_hbm, wu_hbm, wd_hbm = (
        r.bitcast(u32) for r in (x_hbm, out_hbm, wqkv_hbm, wo_hbm, wg_hbm, wu_hbm, wd_hbm))

    def cp_x(lo, hi, extra=()):
        rws = pl.ds(lo * (TB // 2), (hi - lo) * (TB // 2))
        return copies([(x_hbm.at[rws, lanes(c)], x_v.at[c, rws]) for c in range(NC)] + list(extra))

    def cp_out(i, c):
        return pltpu.make_async_copy(out_v.at[c, rows(i)], out_hbm.at[rows(i), lanes(c)],
                                     sems.at[0])

    def slab(i, u):
        return pl.ds(i * (TB // 2) + u, 64, stride=NU)

    def load_rows(ref, rws=slice(None)):
        return jnp.concatenate([ref[c, rws, :] for c in range(ref.shape[0])], axis=1)

    def load_bf16(ref, rws=slice(None)):
        return pltpu.bitcast(load_rows(ref, rws), bf16)

    def store_bf16(ref, rws, val):
        val = pltpu.bitcast(val.astype(bf16), u32)
        for c in range(ref.shape[0]):
            ref[c, rws, :] = val[:, c * 128:(c + 1) * 128]

    def head_major_rows(base, d):
        return pl.ds(base + d, 8, stride=DH)

    wT, woT, xT, gate, oT = {}, {}, {}, {}, {}
    w_ready = set()

    def prep_qkv(p, g):
        base = p * D + g * GR
        for t in range(base // 128, (base + GR - 1) // 128 + 1):
            if t not in w_ready:
                w_ready.add(t)
                for c in range(NC):
                    tmp[c, lanes(t), :] = pltpu.bitcast(
                        wqkv_v[pl.ds(c * 64, 64), lanes(t)], bf16).astype(f32).T
                    yield 60
        parts = []
        for d in range(0, DH, 2):
            two = jnp.concatenate([load_rows(tmp, head_major_rows(base, d)),
                                   load_rows(tmp, head_major_rows(base, d + 1))], axis=0)
            parts.append(two.astype(bf16))
            yield 30
        wT[p, g] = jnp.concatenate(parts, axis=0)

    def prep_wo():
        for c in range(NC):
            perm = jnp.concatenate(
                [wo_v[c, pl.ds(g * GR // 2 + dp, 8, stride=DH // 2), :]
                 for g in range(HG) for dp in range(DH // 2)], axis=0)
            woT[c] = pltpu.bitcast(perm, bf16).T
            yield 200

    def prep_x(i):
        for u in range(NU):
            cols = []
            for c in range(NC):
                cols.append(pltpu.bitcast(x_v[c, slab(i, u), :], bf16).T)
            xT[i, u] = jnp.concatenate(cols, axis=0)
            yield 201

    def router(i):
        wr = wr_ref[...].astype(f32).reshape(1, D)
        for u in range(NU):
            acc_r = None
            for c in range(NC):
                xs = pltpu.bitcast(x_v[c, slab(i, u), :], bf16).astype(f32)
                term = xs * wr[:, c * 128:(c + 1) * 128]
                acc_r = term if c == 0 else acc_r + term
                yield 50
            score_s[pl.ds(i * NU + u, 1), :] = jnp.sum(acc_r.T, axis=0, keepdims=True)
            yield 50

    lane = lax.broadcasted_iota(jnp.int32, (1, 128), 1)
    query, raw, logit, prob, inv, acc = {}, {}, {}, {}, {}, {}

    def taps(p, i, g, t, d, cur):
        prev = raw.pop((p, g, t, d)) if i > 0 else 0.0
        if i + 1 < NB:
            raw[p, g, t, d] = cur
        for wrap in range((W - 1 + NU - 1) // NU + 1):
            us = [u for u in range(NU) if 0 <= u - t + wrap * NU < W]
            if us:
                x = cur if wrap == 0 else pltpu.roll(
                    jnp.where(lane >= 128 - 2 * wrap, prev, cur), 2 * wrap, 1)
                for u in us:
                    yield u, u - t + wrap * NU, x

    def scores(i, g, t, k):
        for d in range(DH):
            for u, w, x in taps(1, i, g, t, d, k[d * 8:(d + 1) * 8]):
                term = query[i, g, u][d * 8:(d + 1) * 8] * x
                logit[u, w] = logit[u, w] + term if d else term

    def softmax(i, g):
        for u in range(NU):
            ls = []
            for w in range(W):
                l = logit.pop((u, w))
                if i == 0 and w > u:
                    l = jnp.where(lane >= 2 * ((w - u + NU - 1) // NU), l, MASKED)
                ls.append(l)
            m = functools.reduce(jnp.maximum, ls)
            for w in range(W):
                prob[u, w] = jnp.exp2((ls[w] - m) * EXP_SCALE)
            inv[u] = 1.0 / functools.reduce(jnp.add, [prob[u, w] for w in range(W)])

    def values(i, g, t, v):
        for d in range(DH):
            for u, w, x in taps(2, i, g, t, d, v[d * 8:(d + 1) * 8]):
                term = prob[u, w] * x
                acc[u, d] = acc[u, d] + term if (u, d) in acc else term
            if t == NU - 1 and d % 2:
                for u in range(NU):
                    pair = [acc.pop((u, d - 1)) * inv[u], acc.pop((u, d)) * inv[u]]
                    oT.setdefault((i, u), []).append(pltpu.bitcast(
                        pltpu.pack_elementwise(pair, packed_dtype=bf16), u32))

    def project(work, ts):
        for i in sorted({i for _, i, _ in work}):
            mine = [(p, g) for p, ii, g in work if ii == i]
            lhs = [wT[pg] for pg in mine]
            if (0, 0) in mine:
                gw = gw_ref[...].astype(f32).reshape(1, D)
                lhs.append(jnp.broadcast_to(gw, (16, D)).astype(bf16))
            r = jnp.dot(jnp.concatenate(lhs, axis=0),
                        jnp.concatenate([xT[i, t] for t in ts], axis=1),
                        preferred_element_type=f32)
            for m, t in enumerate(ts):
                rt = r[:, m * 128:(m + 1) * 128]
                if (0, 0) in mine:
                    gt = jax.nn.sigmoid(rt[len(mine) * GR:len(mine) * GR + 8])
                    gate[i, t] = jnp.tile(gt, (16, 1)).T
                for n, (p, g) in enumerate(mine):
                    part = rt[n * GR:(n + 1) * GR]
                    if p == 0:
                        query[i, g, t] = part
                    else:
                        (scores, values)[p - 1](i, g, t, part)

    jobs, slow = [], []

    def background(budget, queue=jobs):
        while queue and budget > 0:
            cost = next(queue[0], None)
            if cost is None:
                queue.pop(0)
            else:
                budget -= cost

    picks = []

    def route():
        r = score_s[...]
        r = r.astype(bf16).astype(f32)
        key = jnp.where(r != r, -jnp.inf, r)
        sub = lax.broadcasted_iota(jnp.int32, (NB * NU, 128), 0)
        pos = (sub // NU) * TB + (lane // 2) * (2 * NU) + (sub % NU) * 2 + lane % 2
        free = pos >= 0
        for _ in range(2):
            m = jnp.max(jnp.where(free, key, -jnp.inf), keepdims=True)
            idx = jnp.min(jnp.where(free & (key == m), pos, S - 1))
            score = jnp.sum(jnp.where(pos == idx, r, 0.0), keepdims=True)
            free = free & (pos != idx)
            picks.append((idx, jax.nn.sigmoid(score)))
            yield 50

    row = lax.broadcasted_iota(jnp.int32, (16, D), 0)
    hidden = []

    def halves(ref, j):
        word = ref[pl.ds(8 * j, 8), :]
        return [pltpu.unpack_elementwise(word, index=n, packed_dtype=bf16, unpacked_dtype=f32)
                for n in range(2)]

    def picked(idx):
        tile = pl.ds(pl.multiple_of((idx // 16) * 8, 8), 8)
        return tile, row == idx % 16, load_bf16(x_v, tile).astype(f32)

    def ffn_hidden():
        xs = []
        for idx, _ in picks:
            _, hit, cur = picked(idx)
            xs.append(jnp.broadcast_to(
                jnp.sum(jnp.where(hit, cur, 0.0), axis=0, keepdims=True), (8, D)))

        def matvec(w, x):
            prod = w * x
            part = functools.reduce(
                jnp.add, [prod[:, c * 128:(c + 1) * 128] for c in range(NC)])
            return jnp.sum(part, axis=1, keepdims=True)

        for j in range(F // 16):
            hs = []
            for wg, wu in zip(halves(wg_v, j), halves(wu_v, j)):
                for x in xs:
                    half = 0.5 * matvec(wg, x)
                    h = (half * jnp.tanh(half) + half) * matvec(wu, x)
                    hs.append(jnp.broadcast_to(h, (8, 128)))
            hidden.append(hs)
            yield 130

    def ffn_out():
        ys = [None] * len(picks)
        for j in range(F // 16):
            for n, wd in enumerate(halves(wd_v, j)):
                for k in range(len(picks)):
                    term = wd * jnp.tile(hidden[j][n * len(picks) + k], (1, NC))
                    ys[k] = term if ys[k] is None else ys[k] + term
            yield 50
        for (idx, weight), y in zip(picks, ys):
            tile, hit, cur = picked(idx)
            y = jnp.sum(y, axis=0, keepdims=True) * weight
            store_bf16(x_v, tile, jnp.where(hit, cur + y, cur))

    def out_proj(i, cs, us):
        rhs = jnp.concatenate(
            [pltpu.bitcast(jnp.concatenate(oT[i, u], axis=0), bf16) for u in us], axis=1)
        aT = jnp.dot(jnp.concatenate([woT[c] for c in cs], axis=0), rhs,
                     preferred_element_type=f32)
        return {(c, u): aT[n * 128:(n + 1) * 128, m * 128:(m + 1) * 128]
                for n, c in enumerate(cs) for m, u in enumerate(us)}

    def mix(i, tiles):
        for (c, u), aT in tiles.items():
            b = pltpu.bitcast(x_v[c, slab(i, u), :], bf16).astype(f32)
            o = gate[i, u] * aT.T + (1.0 - gate[i, u]) * b
            out_v[c, slab(i, u), :] = pltpu.bitcast(o.astype(bf16), u32)
            if u == NU - 1 and (i == NB - 1 or not CFG["bulk"]):
                cp_out(i, c).start()
            elif (u, c) == (NU - 1, NC - 1):
                start([cp_out(i, n) for n in range(NC)])

    def scope(name):
        return jax.named_scope("@" + name) if CFG["scopes"] else contextlib.nullcontext()

    n_groups = NB * HG
    steps = [[(p, n // HG, n % HG) for p, n in CFG["order"](s) if 0 <= n < n_groups]
             for s in range(-1, n_groups + 1)]

    def w_tiles(work):
        return [t for p, i, g in work
                for t in range((p * D + g * GR) // 128, (p * D + g * GR + GR - 1) // 128 + 1)]

    seen = set()

    def w_pairs(lo, hi):
        new = [t for work in steps[lo:hi] for t in w_tiles(work)]
        new = [t for t in dict.fromkeys(new) if t not in seen]
        seen.update(new)
        runs = [[t for _, t in run] for _, run in
                itertools.groupby(enumerate(sorted(new)), lambda nt: nt[1] - nt[0])]
        cols = [pl.ds(run[0] * 128, len(run) * 128) for run in runs]
        return [(wqkv_hbm.at[:, cl], wqkv_v.at[:, cl]) for cl in cols]

    batch = dict(w0=copies(w_pairs(0, 1)), w1=copies(w_pairs(1, 2)), w2=copies(w_pairs(2, 3)),
                 w3=copies(w_pairs(3, CFG["w3"])),
                 x0=cp_x(0, 1, [(gw_hbm, gw_ref), (wr_hbm, wr_ref)]), x1=cp_x(1, 2, w_pairs(3, len(steps))), x2=cp_x(2, NB),
                 gu=copies([(wg_hbm, wg_v), (wu_hbm, wu_v)]),
                 rest=copies([(wd_hbm, wd_v)] +
                             [(wo_hbm.at[:, lanes(c)], wo_v.at[c]) for c in range(NC)]))
    flying = []

    def run(actions):
        cost = 0
        for act, arg in actions:
            if act == "start":
                start(batch[arg])
                flying.append(arg)
            elif act == "wait":
                with scope(arg):
                    wait(batch[arg])
                flying.remove(arg)
            elif act == "w":
                for p, i, g in steps[arg]:
                    if i == 0:
                        jobs.append(prep_qkv(p, g))
                        cost += 700
            else:
                job, c = dict(x=(prep_x, 800), router=(router, 1200), wo=(prep_wo, 1000),
                              route=(route, 100), hidden=(ffn_hidden, 0), out=(ffn_out, 0))[act]
                (slow if act in ("hidden", "out") else jobs).append(job(*arg))
                cost += c
        return cost

    for actions, budget in CFG["head"]:
        run(actions)
        background(budget)
    for s, work in enumerate(steps):
        with contextlib.nullcontext():
            cost = 0 if s else 600
            nu = CFG["nu"] if s >= CFG["nu_from"] else 1
            for t in range(0, NU, nu):
                cost += run(CFG["events"].get((s, t), ()))
                project(work, range(t, t + nu))
                share = cost * nu / (NU - t)
                background(share)
                cost -= share
                background(CFG["slow"].get(s, 0) * nu / NU, slow)
            background(1e9)
            for p, i, g in work:
                if p == 1:
                    softmax(i, g)
        if s == CFG.get("stop"):
            out_v[0, 0:8, :] = pltpu.bitcast(functools.reduce(
                jnp.add, list(prob.values()) + list(inv.values()) + [v[:8] for v in query.values()]), u32)
            for ws in oT.values():
                for k, word in enumerate(ws):
                    out_v[1, pl.ds(8 * k, 8), :] = word
            wait([c for nm in flying for c in batch[nm]])
            cp_out(0, 0).start()
            cp_out(0, 0).wait()
            return
    pieces = [(i, cs, us) for i in range(NB)
              for cs, us in CFG["last" if i == NB - 1 else "cs"]]
    held = []
    for n, (i, cs, us) in enumerate(pieces):
        held.append((i, out_proj(i, cs, us)))
        if n < CFG["hold"]:
            background(CFG["slow_c"] * len(cs), slow)
            continue
        background(1e9, slow)
        for _ in range(2):
            if held:
                mix(*held.pop(0))
    for piece in held:
        mix(*piece)
    with scope("out"):
        wait([cp_out(i, c) for i in range(NB) for c in range(NC)])


@jax.jit
def pallas_gated_mix__sliding_local_dilated__moe_arch_mod__prompt_kernel(
    A_x: jax.Array,
    A_wqkv: jax.Array,
    A_wo: jax.Array,
    B_x: jax.Array,
    B_w_r: jax.Array,
    B_w_gate: jax.Array,
    B_w_up: jax.Array,
    B_w_down: jax.Array,
    gate_w: jax.Array,
):
    hbm = pl.BlockSpec(memory_space=pl.ANY)
    return pl.pallas_call(
        _kernel,
        out_shape=jax.ShapeDtypeStruct((S, D), A_x.dtype),
        in_specs=[hbm] * 8,
        out_specs=hbm,
        interpret=CFG["interpret"],
        scratch_shapes=[
            pltpu.VMEM((NC, S // 2, 128), u32),
            pltpu.VMEM((D // 2, 3 * D), u32),
            pltpu.VMEM((NC, D // 2, 128), u32),
            pltpu.VMEM((F // 2, D), u32),
            pltpu.VMEM((F // 2, D), u32),
            pltpu.VMEM((F // 2, D), u32),
            pltpu.VMEM((NC, S // 2, 128), u32),
            pltpu.VMEM((NC, 3 * D, 128), f32),
            pltpu.VMEM((NB * NU, 128), f32),
            pltpu.VMEM((D,), bf16),
            pltpu.VMEM((D,), bf16),
            pltpu.SemaphoreType.DMA((N_SEMS,)),
        ],
        compiler_params=pltpu.CompilerParams(
            vmem_limit_bytes=100 * 1024 * 1024, flags=CFG["flags"]),
    )(A_x.reshape(S, D), A_wqkv, A_wo, B_w_r, B_w_gate.T, B_w_up.T, B_w_down,
      gate_w).reshape(A_x.shape)
```

```python
import contextlib
import functools
import itertools
import math

import jax
import jax.numpy as jnp
from jax import lax
import jax.experimental.pallas as pl
import jax.experimental.pallas.tpu as pltpu

CFG = dict(
    flags=None, interpret=False, scopes=False,
    head=(([("start", "w0"), ("start", "x0"), ("wait", "w0"), ("start", "w1"), ("w", (0, 0, 3))], 1e9),
          ([("wait", "x0"), ("start", "w2"), ("x", (0,))], 201)),
    nu=1, nu_from=5,
    events={
        (0, 1): [("wait", "w1"), ("start", "w3"), ("w", (1, 0, 3))],
        (1, 0): [("w", (2, 0, 3))],
        (2, 1): [("wait", "w2"), ("start", "x1"), ("w", (3, 0, 3))],
        (3, 0): [("w", (4, 0, 3)), ("w", (5, 0, 3))],
        (4, 0): [("wait", "w3"), ("start", "x2"), ("w", (6, 0, 1))],
        (5, 0): [("w", (6, 1, 3))],
        (6, 0): [("wait", "x1"), ("w", (7, 0, 3)), ("x", (1,))],
        (7, 0): [("wait", "x2"), ("start", "gu"), ("start", "rest"), ("w", (8, 0, 3))],
        (8, 0): [("router", (0,)), ("router", (1,))],
        (9, 0): [("router", (2,))],
        (10, 0): [("x", (2,))],
        (11, 0): [("router", (3,))],
        (12, 0): [("route", ())],
        (13, 0): [("wait", "gu"), ("wait", "rest"), ("hidden", ()), ("out", ())],
        (14, 0): [("x", (3,))],
        (17, 0): [("wo", ())],
    },
    slow={13: 3600, 14: 3200, 15: 3600, 16: 3600, 17: 3200, 18: 3000},
    hold=0, bulk=True, w3=4, slow_c=800,
    order=lambda s: ((1, s), (2, s - 1), (0, s + 1)),
    cs=[((0, 1, 2, 3, 4), (0, 1)), ((0, 1, 2, 3, 4), (2, 3))],
    last=[((0, 1, 2), (0, 1)), ((0, 1, 2), (2, 3)), ((3,), (0, 1, 2, 3)),
          ((4,), (0, 1)), ((4,), (2,)), ((4,), (3,))])

S, D, H, F = 2048, 640, 32, 1728
DH = D // H
W = 8
HG = H // 8
GR = 8 * DH
TB = 512
NB = S // TB
NU = TB // 128
NC = D // 128
NE = W - 1
N_SEMS = 10
SCALE = DH ** -0.5
EXP_SCALE = SCALE * math.log2(math.e)
MASKED = -1e9 / SCALE

f32, bf16, u32 = jnp.float32, jnp.bfloat16, jnp.uint32
NT = (((1,), (1,)), ((), ()))


def _kernel(x_hbm, wqkv_hbm, wo_hbm, wr_hbm, wg_hbm, wu_hbm, wd_hbm, gw_hbm,
            out_hbm,
            x_v, wqkv_v, wo_v, wg_v, wu_v, wd_v, out_v,
            tmp, score_s, wr_ref, gw_ref, sems):
    free_sems = iter(range(1, N_SEMS))

    def copies(pairs):
        sem = sems.at[next(free_sems)]
        return [pltpu.make_async_copy(src, dst, sem) for src, dst in pairs]

    def start(cps):
        for c in cps:
            c.start()

    def wait(cps):
        for c in cps:
            c.wait()

    def rows(i):
        return pl.ds(pl.multiple_of(i * (TB // 2), TB // 2), TB // 2)

    def lanes(c):
        return pl.ds(c * 128, 128)

    x_hbm, out_hbm, wqkv_hbm, wo_hbm, wg_hbm, wu_hbm, wd_hbm = (
        r.bitcast(u32) for r in (x_hbm, out_hbm, wqkv_hbm, wo_hbm, wg_hbm, wu_hbm, wd_hbm))

    def cp_x(lo, hi, extra=()):
        rws = pl.ds(lo * (TB // 2), (hi - lo) * (TB // 2))
        return copies([(x_hbm.at[rws, lanes(c)], x_v.at[c, rws]) for c in range(NC)] + list(extra))

    def cp_out(i, c):
        return pltpu.make_async_copy(out_v.at[c, rows(i)], out_hbm.at[rows(i), lanes(c)],
                                     sems.at[0])

    def slab(i, u):
        return pl.ds(i * (TB // 2) + u, 64, stride=NU)

    def load_rows(ref, rws=slice(None)):
        return jnp.concatenate([ref[c, rws, :] for c in range(ref.shape[0])], axis=1)

    def load_bf16(ref, rws=slice(None)):
        return pltpu.bitcast(load_rows(ref, rws), bf16)

    def store_bf16(ref, rws, val):
        val = pltpu.bitcast(val.astype(bf16), u32)
        for c in range(ref.shape[0]):
            ref[c, rws, :] = val[:, c * 128:(c + 1) * 128]

    def head_major_rows(base, d):
        return pl.ds(base + d, 8, stride=DH)

    wT, woT, xT, gate, oT = {}, {}, {}, {}, {}
    w_ready = set()

    def prep_qkv(p, g):
        base = p * D + g * GR
        for t in range(base // 128, (base + GR - 1) // 128 + 1):
            if t not in w_ready:
                w_ready.add(t)
                for c in range(NC):
                    tmp[c, lanes(t), :] = pltpu.bitcast(
                        wqkv_v[pl.ds(c * 64, 64), lanes(t)], bf16).astype(f32).T
                    yield 60
        parts = []
        for d in range(0, DH, 2):
            two = jnp.concatenate([load_rows(tmp, head_major_rows(base, d)),
                                   load_rows(tmp, head_major_rows(base, d + 1))], axis=0)
            parts.append(two.astype(bf16))
            yield 30
        wT[p, g] = jnp.concatenate(parts, axis=0)

    def prep_wo():
        for c in range(NC):
            perm = jnp.concatenate(
                [wo_v[c, pl.ds(g * GR // 2 + dp, 8, stride=DH // 2), :]
                 for g in range(HG) for dp in range(DH // 2)], axis=0)
            woT[c] = pltpu.bitcast(perm, bf16).T
            yield 200

    def prep_x(i):
        for u in range(NU):
            cols = []
            for c in range(NC):
                cols.append(pltpu.bitcast(x_v[c, slab(i, u), :], bf16).T)
            xT[i, u] = jnp.concatenate(cols, axis=0)
            yield 201

    def router(i):
        wr = wr_ref[...].astype(f32).reshape(1, D)
        for u in range(NU):
            acc_r = None
            for c in range(NC):
                xs = pltpu.bitcast(x_v[c, slab(i, u), :], bf16).astype(f32)
                term = xs * wr[:, c * 128:(c + 1) * 128]
                acc_r = term if c == 0 else acc_r + term
                yield 50
            score_s[pl.ds(i * NU + u, 1), :] = jnp.sum(acc_r.T, axis=0, keepdims=True)
            yield 50

    lane = lax.broadcasted_iota(jnp.int32, (1, 128), 1)
    query, raw, logit, prob, inv, acc = {}, {}, {}, {}, {}, {}

    def taps(p, i, g, t, d, cur):
        prev = raw.pop((p, g, t, d)) if i > 0 else 0.0
        if i + 1 < NB:
            raw[p, g, t, d] = cur
        for wrap in range((W - 1 + NU - 1) // NU + 1):
            us = [u for u in range(NU) if 0 <= u - t + wrap * NU < W]
            if us:
                x = cur if wrap == 0 else pltpu.roll(
                    jnp.where(lane >= 128 - 2 * wrap, prev, cur), 2 * wrap, 1)
                for u in us:
                    yield u, u - t + wrap * NU, x

    def scores(i, g, t, k):
        for d in range(DH):
            for u, w, x in taps(1, i, g, t, d, k[d * 8:(d + 1) * 8]):
                term = query[i, g, u][d * 8:(d + 1) * 8] * x
                logit[u, w] = logit[u, w] + term if d else term

    def softmax(i, g):
        for u in range(NU):
            ls = []
            for w in range(W):
                l = logit.pop((u, w))
                if i == 0 and w > u:
                    l = jnp.where(lane >= 2 * ((w - u + NU - 1) // NU), l, MASKED)
                ls.append(l)
            m = functools.reduce(jnp.maximum, ls)
            for w in range(W):
                prob[u, w] = jnp.exp2((ls[w] - m) * EXP_SCALE)
            inv[u] = 1.0 / functools.reduce(jnp.add, [prob[u, w] for w in range(W)])

    def values(i, g, t, v):
        for d in range(DH):
            for u, w, x in taps(2, i, g, t, d, v[d * 8:(d + 1) * 8]):
                term = prob[u, w] * x
                acc[u, d] = acc[u, d] + term if (u, d) in acc else term
            if t == NU - 1 and d % 2:
                for u in range(NU):
                    pair = [acc.pop((u, d - 1)) * inv[u], acc.pop((u, d)) * inv[u]]
                    oT.setdefault((i, u), []).append(pltpu.bitcast(
                        pltpu.pack_elementwise(pair, packed_dtype=bf16), u32))

    def project(work, ts):
        for i in sorted({i for _, i, _ in work}):
            mine = [(p, g) for p, ii, g in work if ii == i]
            lhs = [wT[pg] for pg in mine]
            if (0, 0) in mine:
                gw = gw_ref[...].astype(f32).reshape(1, D)
                lhs.append(jnp.broadcast_to(gw, (16, D)).astype(bf16))
            r = jnp.dot(jnp.concatenate(lhs, axis=0),
                        jnp.concatenate([xT[i, t] for t in ts], axis=1),
                        preferred_element_type=f32)
            for m, t in enumerate(ts):
                rt = r[:, m * 128:(m + 1) * 128]
                if (0, 0) in mine:
                    gt = jax.nn.sigmoid(rt[len(mine) * GR:len(mine) * GR + 8])
                    gate[i, t] = jnp.tile(gt, (16, 1)).T
                for n, (p, g) in enumerate(mine):
                    part = rt[n * GR:(n + 1) * GR]
                    if p == 0:
                        query[i, g, t] = part
                    else:
                        (scores, values)[p - 1](i, g, t, part)

    jobs, slow = [], []

    def background(budget, queue=jobs):
        while queue and budget > 0:
            cost = next(queue[0], None)
            if cost is None:
                queue.pop(0)
            else:
                budget -= cost

    picks = []

    def route():
        r = score_s[...]
        r = r.astype(bf16).astype(f32)
        key = jnp.where(r != r, -jnp.inf, r)
        sub = lax.broadcasted_iota(jnp.int32, (NB * NU, 128), 0)
        pos = (sub // NU) * TB + (lane // 2) * (2 * NU) + (sub % NU) * 2 + lane % 2
        free = pos >= 0
        for _ in range(2):
            m = jnp.max(jnp.where(free, key, -jnp.inf), keepdims=True)
            idx = jnp.min(jnp.where(free & (key == m), pos, S - 1))
            score = jnp.sum(jnp.where(pos == idx, r, 0.0), keepdims=True)
            free = free & (pos != idx)
            picks.append((idx, jax.nn.sigmoid(score)))
            yield 50

    row = lax.broadcasted_iota(jnp.int32, (16, D), 0)
    hidden = []

    def halves(ref, j):
        word = ref[pl.ds(8 * j, 8), :]
        return [pltpu.unpack_elementwise(word, index=n, packed_dtype=bf16, unpacked_dtype=f32)
                for n in range(2)]

    def picked(idx):
        tile = pl.ds(pl.multiple_of((idx // 16) * 8, 8), 8)
        return tile, row == idx % 16, load_bf16(x_v, tile).astype(f32)

    def ffn_hidden():
        xs = []
        for idx, _ in picks:
            _, hit, cur = picked(idx)
            xs.append(jnp.broadcast_to(
                jnp.sum(jnp.where(hit, cur, 0.0), axis=0, keepdims=True), (8, D)))

        def matvec(w, x):
            prod = w * x
            part = functools.reduce(
                jnp.add, [prod[:, c * 128:(c + 1) * 128] for c in range(NC)])
            return jnp.sum(part, axis=1, keepdims=True)

        for j in range(F // 16):
            hs = []
            for wg, wu in zip(halves(wg_v, j), halves(wu_v, j)):
                for x in xs:
                    half = 0.5 * matvec(wg, x)
                    h = (half * jnp.tanh(half) + half) * matvec(wu, x)
                    hs.append(jnp.broadcast_to(h, (8, 128)))
            hidden.append(hs)
            yield 130

    def ffn_out():
        ys = [None] * len(picks)
        for j in range(F // 16):
            for n, wd in enumerate(halves(wd_v, j)):
                for k in range(len(picks)):
                    term = wd * jnp.tile(hidden[j][n * len(picks) + k], (1, NC))
                    ys[k] = term if ys[k] is None else ys[k] + term
            yield 50
        for (idx, weight), y in zip(picks, ys):
            tile, hit, cur = picked(idx)
            y = jnp.sum(y, axis=0, keepdims=True) * weight
            store_bf16(x_v, tile, jnp.where(hit, cur + y, cur))

    def out_proj(i, cs, us):
        rhs = jnp.concatenate(
            [pltpu.bitcast(jnp.concatenate(oT[i, u], axis=0), bf16) for u in us], axis=1)
        aT = jnp.dot(jnp.concatenate([woT[c] for c in cs], axis=0), rhs,
                     preferred_element_type=f32)
        return {(c, u): aT[n * 128:(n + 1) * 128, m * 128:(m + 1) * 128]
                for n, c in enumerate(cs) for m, u in enumerate(us)}

    def mix(i, tiles):
        for (c, u), aT in tiles.items():
            b = pltpu.bitcast(x_v[c, slab(i, u), :], bf16).astype(f32)
            o = gate[i, u] * aT.T + (1.0 - gate[i, u]) * b
            out_v[c, slab(i, u), :] = pltpu.bitcast(o.astype(bf16), u32)
            if u == NU - 1 and (i == NB - 1 or not CFG["bulk"]):
                cp_out(i, c).start()
            elif (u, c) == (NU - 1, NC - 1):
                start([cp_out(i, n) for n in range(NC)])

    def scope(name):
        return jax.named_scope("@" + name) if CFG["scopes"] else contextlib.nullcontext()

    n_groups = NB * HG
    steps = [[(p, n // HG, n % HG) for p, n in CFG["order"](s) if 0 <= n < n_groups]
             for s in range(-1, n_groups + 1)]
    steps[:3] = [[item] for item in sorted(steps[0]) + sorted(steps[1])[::-1] + sorted(steps[2])[::-1]]

    def w_tiles(work):
        return [t for p, i, g in work
                for t in range((p * D + g * GR) // 128, (p * D + g * GR + GR - 1) // 128 + 1)]

    seen = set()

    def w_pairs(lo, hi):
        new = [t for work in steps[lo:hi] for t in w_tiles(work)]
        new = [t for t in dict.fromkeys(new) if t not in seen]
        seen.update(new)
        runs = [[t for _, t in run] for _, run in
                itertools.groupby(enumerate(sorted(new)), lambda nt: nt[1] - nt[0])]
        cols = [pl.ds(run[0] * 128, len(run) * 128) for run in runs]
        return [(wqkv_hbm.at[:, cl], wqkv_v.at[:, cl]) for cl in cols]

    batch = dict(w0=copies(w_pairs(0, 1)), w1=copies(w_pairs(1, 3)), w2=copies(w_pairs(3, 6)),
                 w3=copies(w_pairs(6, 7)),
                 x0=cp_x(0, 1, [(gw_hbm, gw_ref), (wr_hbm, wr_ref)]), x1=cp_x(1, 2, w_pairs(7, len(steps))), x2=cp_x(2, NB),
                 gu=copies([(wg_hbm, wg_v), (wu_hbm, wu_v)]),
                 rest=copies([(wd_hbm, wd_v)] +
                             [(wo_hbm.at[:, lanes(c)], wo_v.at[c]) for c in range(NC)]))
    flying = []

    def run(actions):
        cost = 0
        for act, arg in actions:
            if act == "start":
                start(batch[arg])
                flying.append(arg)
            elif act == "wait":
                with scope(arg):
                    wait(batch[arg])
                flying.remove(arg)
            elif act == "w":
                for p, i, g in steps[arg[0]][arg[1]:arg[2]]:
                    if i == 0:
                        jobs.append(prep_qkv(p, g))
                        cost += 700
            else:
                job, c = dict(x=(prep_x, 800), router=(router, 1200), wo=(prep_wo, 1000),
                              route=(route, 100), hidden=(ffn_hidden, 0), out=(ffn_out, 0))[act]
                (slow if act in ("hidden", "out") else jobs).append(job(*arg))
                cost += c
        return cost

    for actions, budget in CFG["head"]:
        run(actions)
        background(budget)
    for s, work in enumerate(steps):
        with contextlib.nullcontext():
            cost = 0 if s else 600
            nu = CFG["nu"] if s >= CFG["nu_from"] else 1
            for t in range(0, NU, nu):
                cost += run(CFG["events"].get((s, t), ()))
                project(work, range(t, t + nu))
                share = cost * nu / (NU - t)
                background(share)
                cost -= share
                background(CFG["slow"].get(s, 0) * nu / NU, slow)
            background(1e9)
            for p, i, g in work:
                if p == 1:
                    softmax(i, g)
        if s == CFG.get("stop"):
            out_v[0, 0:8, :] = pltpu.bitcast(functools.reduce(
                jnp.add, list(prob.values()) + list(inv.values()) + [v[:8] for v in query.values()]), u32)
            for ws in oT.values():
                for k, word in enumerate(ws):
                    out_v[1, pl.ds(8 * k, 8), :] = word
            wait([c for nm in flying for c in batch[nm]])
            cp_out(0, 0).start()
            cp_out(0, 0).wait()
            return
    pieces = [(i, cs, us) for i in range(NB)
              for cs, us in CFG["last" if i == NB - 1 else "cs"]]
    held = []
    for n, (i, cs, us) in enumerate(pieces):
        held.append((i, out_proj(i, cs, us)))
        if n < CFG["hold"]:
            background(CFG["slow_c"] * len(cs), slow)
            continue
        background(1e9, slow)
        for _ in range(2):
            if held:
                mix(*held.pop(0))
    for piece in held:
        mix(*piece)
    with scope("out"):
        wait([cp_out(i, c) for i in range(NB) for c in range(NC)])


@jax.jit
def pallas_gated_mix__sliding_local_dilated__moe_arch_mod__prompt_kernel(
    A_x: jax.Array,
    A_wqkv: jax.Array,
    A_wo: jax.Array,
    B_x: jax.Array,
    B_w_r: jax.Array,
    B_w_gate: jax.Array,
    B_w_up: jax.Array,
    B_w_down: jax.Array,
    gate_w: jax.Array,
):
    hbm = pl.BlockSpec(memory_space=pl.ANY)
    return pl.pallas_call(
        _kernel,
        out_shape=jax.ShapeDtypeStruct((S, D), A_x.dtype),
        in_specs=[hbm] * 8,
        out_specs=hbm,
        interpret=CFG["interpret"],
        scratch_shapes=[
            pltpu.VMEM((NC, S // 2, 128), u32),
            pltpu.VMEM((D // 2, 3 * D), u32),
            pltpu.VMEM((NC, D // 2, 128), u32),
            pltpu.VMEM((F // 2, D), u32),
            pltpu.VMEM((F // 2, D), u32),
            pltpu.VMEM((F // 2, D), u32),
            pltpu.VMEM((NC, S // 2, 128), u32),
            pltpu.VMEM((NC, 3 * D, 128), f32),
            pltpu.VMEM((NB * NU, 128), f32),
            pltpu.VMEM((D,), bf16),
            pltpu.VMEM((D,), bf16),
            pltpu.SemaphoreType.DMA((N_SEMS,)),
        ],
        compiler_params=pltpu.CompilerParams(
            vmem_limit_bytes=100 * 1024 * 1024, flags=CFG["flags"]),
    )(A_x.reshape(S, D), A_wqkv, A_wo, B_w_r, B_w_gate.T, B_w_up.T, B_w_down,
      gate_w).reshape(A_x.shape)
```

```python
import functools
import itertools
import math

import jax
import jax.numpy as jnp
from jax import lax
import jax.experimental.pallas as pl
import jax.experimental.pallas.tpu as pltpu

S, D, H, F = 2048, 640, 32, 1728
DH = D // H
W = 8
HG = H // 8
GR = 8 * DH
TB = 512
NB = S // TB
NU = TB // 128
NC = D // 128
NE = W - 1
N_SEMS = 10
SCALE = DH ** -0.5
EXP_SCALE = SCALE * math.log2(math.e)
MASKED = -1e9 / SCALE

HEAD = (
    ([("start", "w0"), ("start", "x0"), ("wait", "w0"), ("start", "w1"), ("w", (0, 0, 3))], 1e9),
    ([("wait", "x0"), ("start", "w2"), ("x", (0,))], 201),
)
EVENTS = {
    (0, 1): [("wait", "w1"), ("start", "w3"), ("w", (1, 0, 3))],
    (1, 0): [("w", (2, 0, 3))],
    (2, 1): [("wait", "w2"), ("start", "x1"), ("w", (3, 0, 3))],
    (3, 0): [("w", (4, 0, 3)), ("w", (5, 0, 3))],
    (4, 0): [("wait", "w3"), ("start", "x2"), ("w", (6, 0, 1))],
    (5, 0): [("w", (6, 1, 3))],
    (6, 0): [("wait", "x1"), ("w", (7, 0, 3)), ("x", (1,))],
    (7, 0): [("wait", "x2"), ("start", "gu"), ("start", "rest"), ("w", (8, 0, 3))],
    (8, 0): [("router", (0,)), ("router", (1,))],
    (9, 0): [("router", (2,))],
    (10, 0): [("x", (2,))],
    (11, 0): [("router", (3,))],
    (12, 0): [("route", ())],
    (13, 0): [("wait", "gu"), ("wait", "rest"), ("hidden", ()), ("out", ())],
    (14, 0): [("x", (3,))],
    (17, 0): [("wo", ())],
}
FFN_BUDGET = {13: 3600, 14: 3200, 15: 3600, 16: 3600, 17: 3200, 18: 3000}
OUT_PIECES = [((0, 1, 2, 3, 4), (0, 1)), ((0, 1, 2, 3, 4), (2, 3))]
LAST_PIECES = [((0, 1, 2), (0, 1)), ((0, 1, 2), (2, 3)), ((3,), (0, 1, 2, 3)),
               ((4,), (0, 1)), ((4,), (2,)), ((4,), (3,))]

f32, bf16, u32 = jnp.float32, jnp.bfloat16, jnp.uint32


def _kernel(x_hbm, wqkv_hbm, wo_hbm, wr_hbm, wg_hbm, wu_hbm, wd_hbm, gw_hbm,
            out_hbm,
            x_v, wqkv_v, wo_v, wg_v, wu_v, wd_v, out_v,
            tmp, score_s, wr_ref, gw_ref, sems):
    free_sems = iter(range(1, N_SEMS))

    def copies(pairs):
        sem = sems.at[next(free_sems)]
        return [pltpu.make_async_copy(src, dst, sem) for src, dst in pairs]

    def start(cps):
        for c in cps:
            c.start()

    def wait(cps):
        for c in cps:
            c.wait()

    def rows(i):
        return pl.ds(pl.multiple_of(i * (TB // 2), TB // 2), TB // 2)

    def lanes(c):
        return pl.ds(c * 128, 128)

    x_hbm, out_hbm, wqkv_hbm, wo_hbm, wg_hbm, wu_hbm, wd_hbm = (
        r.bitcast(u32) for r in (x_hbm, out_hbm, wqkv_hbm, wo_hbm, wg_hbm, wu_hbm, wd_hbm))

    def cp_x(lo, hi, extra=()):
        rws = pl.ds(lo * (TB // 2), (hi - lo) * (TB // 2))
        return copies([(x_hbm.at[rws, lanes(c)], x_v.at[c, rws]) for c in range(NC)] + list(extra))

    def cp_out(i, c):
        return pltpu.make_async_copy(out_v.at[c, rows(i)], out_hbm.at[rows(i), lanes(c)],
                                     sems.at[0])

    def slab(i, u):
        return pl.ds(i * (TB // 2) + u, 64, stride=NU)

    def load_rows(ref, rws=slice(None)):
        return jnp.concatenate([ref[c, rws, :] for c in range(ref.shape[0])], axis=1)

    def load_bf16(ref, rws=slice(None)):
        return pltpu.bitcast(load_rows(ref, rws), bf16)

    def store_bf16(ref, rws, val):
        val = pltpu.bitcast(val.astype(bf16), u32)
        for c in range(ref.shape[0]):
            ref[c, rws, :] = val[:, c * 128:(c + 1) * 128]

    def head_major_rows(base, d):
        return pl.ds(base + d, 8, stride=DH)

    wT, woT, xT, gate, oT = {}, {}, {}, {}, {}
    w_ready = set()

    def prep_qkv(p, g):
        base = p * D + g * GR
        for t in range(base // 128, (base + GR - 1) // 128 + 1):
            if t not in w_ready:
                w_ready.add(t)
                for c in range(NC):
                    tmp[c, lanes(t), :] = pltpu.bitcast(
                        wqkv_v[pl.ds(c * 64, 64), lanes(t)], bf16).astype(f32).T
                    yield 60
        parts = []
        for d in range(0, DH, 2):
            two = jnp.concatenate([load_rows(tmp, head_major_rows(base, d)),
                                   load_rows(tmp, head_major_rows(base, d + 1))], axis=0)
            parts.append(two.astype(bf16))
            yield 30
        wT[p, g] = jnp.concatenate(parts, axis=0)

    def prep_wo():
        for c in range(NC):
            perm = jnp.concatenate(
                [wo_v[c, pl.ds(g * GR // 2 + dp, 8, stride=DH // 2), :]
                 for g in range(HG) for dp in range(DH // 2)], axis=0)
            woT[c] = pltpu.bitcast(perm, bf16).T
            yield 200

    def prep_x(i):
        for u in range(NU):
            cols = []
            for c in range(NC):
                cols.append(pltpu.bitcast(x_v[c, slab(i, u), :], bf16).T)
            xT[i, u] = jnp.concatenate(cols, axis=0)
            yield 201

    def router(i):
        wr = wr_ref[...].astype(f32).reshape(1, D)
        for u in range(NU):
            acc_r = None
            for c in range(NC):
                xs = pltpu.bitcast(x_v[c, slab(i, u), :], bf16).astype(f32)
                term = xs * wr[:, c * 128:(c + 1) * 128]
                acc_r = term if c == 0 else acc_r + term
                yield 50
            score_s[pl.ds(i * NU + u, 1), :] = jnp.sum(acc_r.T, axis=0, keepdims=True)
            yield 50

    lane = lax.broadcasted_iota(jnp.int32, (1, 128), 1)
    query, raw, logit, prob, inv, acc = {}, {}, {}, {}, {}, {}

    def taps(p, i, g, t, d, cur):
        prev = raw.pop((p, g, t, d)) if i > 0 else 0.0
        if i + 1 < NB:
            raw[p, g, t, d] = cur
        for wrap in range((W - 1 + NU - 1) // NU + 1):
            us = [u for u in range(NU) if 0 <= u - t + wrap * NU < W]
            if us:
                x = cur if wrap == 0 else pltpu.roll(
                    jnp.where(lane >= 128 - 2 * wrap, prev, cur), 2 * wrap, 1)
                for u in us:
                    yield u, u - t + wrap * NU, x

    def scores(i, g, t, k):
        for d in range(DH):
            for u, w, x in taps(1, i, g, t, d, k[d * 8:(d + 1) * 8]):
                term = query[i, g, u][d * 8:(d + 1) * 8] * x
                logit[u, w] = logit[u, w] + term if d else term

    def softmax(i, g):
        for u in range(NU):
            ls = []
            for w in range(W):
                l = logit.pop((u, w))
                if i == 0 and w > u:
                    l = jnp.where(lane >= 2 * ((w - u + NU - 1) // NU), l, MASKED)
                ls.append(l)
            m = functools.reduce(jnp.maximum, ls)
            for w in range(W):
                prob[u, w] = jnp.exp2((ls[w] - m) * EXP_SCALE)
            inv[u] = 1.0 / functools.reduce(jnp.add, [prob[u, w] for w in range(W)])

    def values(i, g, t, v):
        for d in range(DH):
            for u, w, x in taps(2, i, g, t, d, v[d * 8:(d + 1) * 8]):
                term = prob[u, w] * x
                acc[u, d] = acc[u, d] + term if (u, d) in acc else term
            if t == NU - 1 and d % 2:
                for u in range(NU):
                    pair = [acc.pop((u, d - 1)) * inv[u], acc.pop((u, d)) * inv[u]]
                    oT.setdefault((i, u), []).append(pltpu.bitcast(
                        pltpu.pack_elementwise(pair, packed_dtype=bf16), u32))

    def project(work, t):
        for i in sorted({i for _, i, _ in work}):
            mine = [(p, g) for p, ii, g in work if ii == i]
            lhs = [wT[pg] for pg in mine]
            if (0, 0) in mine:
                gw = gw_ref[...].astype(f32).reshape(1, D)
                lhs.append(jnp.broadcast_to(gw, (16, D)).astype(bf16))
            r = jnp.dot(jnp.concatenate(lhs, axis=0), xT[i, t], preferred_element_type=f32)
            if (0, 0) in mine:
                gt = jax.nn.sigmoid(r[len(mine) * GR:len(mine) * GR + 8])
                gate[i, t] = jnp.tile(gt, (16, 1)).T
            for n, (p, g) in enumerate(mine):
                part = r[n * GR:(n + 1) * GR]
                if p == 0:
                    query[i, g, t] = part
                else:
                    (scores, values)[p - 1](i, g, t, part)

    jobs, slow = [], []

    def background(budget, queue=jobs):
        while queue and budget > 0:
            cost = next(queue[0], None)
            if cost is None:
                queue.pop(0)
            else:
                budget -= cost

    picks = []

    def route():
        r = score_s[...]
        r = r.astype(bf16).astype(f32)
        key = jnp.where(r != r, -jnp.inf, r)
        sub = lax.broadcasted_iota(jnp.int32, (NB * NU, 128), 0)
        pos = (sub // NU) * TB + (lane // 2) * (2 * NU) + (sub % NU) * 2 + lane % 2
        free = pos >= 0
        for _ in range(2):
            m = jnp.max(jnp.where(free, key, -jnp.inf), keepdims=True)
            idx = jnp.min(jnp.where(free & (key == m), pos, S - 1))
            score = jnp.sum(jnp.where(pos == idx, r, 0.0), keepdims=True)
            free = free & (pos != idx)
            picks.append((idx, jax.nn.sigmoid(score)))
            yield 50

    row = lax.broadcasted_iota(jnp.int32, (16, D), 0)
    hidden = []

    def halves(ref, j):
        word = ref[pl.ds(8 * j, 8), :]
        return [pltpu.unpack_elementwise(word, index=n, packed_dtype=bf16, unpacked_dtype=f32)
                for n in range(2)]

    def picked(idx):
        tile = pl.ds(pl.multiple_of((idx // 16) * 8, 8), 8)
        return tile, row == idx % 16, load_bf16(x_v, tile).astype(f32)

    def ffn_hidden():
        xs = []
        for idx, _ in picks:
            _, hit, cur = picked(idx)
            xs.append(jnp.broadcast_to(
                jnp.sum(jnp.where(hit, cur, 0.0), axis=0, keepdims=True), (8, D)))

        def matvec(w, x):
            prod = w * x
            part = functools.reduce(
                jnp.add, [prod[:, c * 128:(c + 1) * 128] for c in range(NC)])
            return jnp.sum(part, axis=1, keepdims=True)

        for j in range(F // 16):
            hs = []
            for wg, wu in zip(halves(wg_v, j), halves(wu_v, j)):
                for x in xs:
                    half = 0.5 * matvec(wg, x)
                    h = (half * jnp.tanh(half) + half) * matvec(wu, x)
                    hs.append(jnp.broadcast_to(h, (8, 128)))
            hidden.append(hs)
            yield 130

    def ffn_out():
        ys = [None] * len(picks)
        for j in range(F // 16):
            for n, wd in enumerate(halves(wd_v, j)):
                for k in range(len(picks)):
                    term = wd * jnp.tile(hidden[j][n * len(picks) + k], (1, NC))
                    ys[k] = term if ys[k] is None else ys[k] + term
            yield 50
        assert len(xT) == NB * NU
        for (idx, weight), y in zip(picks, ys):
            tile, hit, cur = picked(idx)
            y = jnp.sum(y, axis=0, keepdims=True) * weight
            store_bf16(x_v, tile, jnp.where(hit, cur + y, cur))

    def out_proj(i, cs, us):
        rhs = jnp.concatenate(
            [pltpu.bitcast(jnp.concatenate(oT[i, u], axis=0), bf16) for u in us], axis=1)
        aT = jnp.dot(jnp.concatenate([woT[c] for c in cs], axis=0), rhs,
                     preferred_element_type=f32)
        return {(c, u): aT[n * 128:(n + 1) * 128, m * 128:(m + 1) * 128]
                for n, c in enumerate(cs) for m, u in enumerate(us)}

    def mix(i, tiles):
        for (c, u), aT in tiles.items():
            b = pltpu.bitcast(x_v[c, slab(i, u), :], bf16).astype(f32)
            o = gate[i, u] * aT.T + (1.0 - gate[i, u]) * b
            out_v[c, slab(i, u), :] = pltpu.bitcast(o.astype(bf16), u32)
            if u == NU - 1 and i == NB - 1:
                cp_out(i, c).start()
            elif (u, c) == (NU - 1, NC - 1):
                start([cp_out(i, n) for n in range(NC)])

    n_groups = NB * HG
    steps = [[(p, n // HG, n % HG) for p, n in ((1, s), (2, s - 1), (0, s + 1)) if 0 <= n < n_groups]
             for s in range(-1, n_groups + 1)]
    steps[:3] = [[item] for item in sorted(steps[0]) + sorted(steps[1])[::-1] + sorted(steps[2])[::-1]]

    def w_tiles(work):
        return [t for p, i, g in work
                for t in range((p * D + g * GR) // 128, (p * D + g * GR + GR - 1) // 128 + 1)]

    seen = set()

    def w_pairs(lo, hi):
        new = [t for work in steps[lo:hi] for t in w_tiles(work)]
        new = [t for t in dict.fromkeys(new) if t not in seen]
        seen.update(new)
        runs = [[t for _, t in run] for _, run in
                itertools.groupby(enumerate(sorted(new)), lambda nt: nt[1] - nt[0])]
        cols = [pl.ds(run[0] * 128, len(run) * 128) for run in runs]
        return [(wqkv_hbm.at[:, cl], wqkv_v.at[:, cl]) for cl in cols]

    batch = dict(w0=copies(w_pairs(0, 1)), w1=copies(w_pairs(1, 3)), w2=copies(w_pairs(3, 6)),
                 w3=copies(w_pairs(6, 7)),
                 x0=cp_x(0, 1, [(gw_hbm, gw_ref), (wr_hbm, wr_ref)]), x1=cp_x(1, 2, w_pairs(7, len(steps))), x2=cp_x(2, NB),
                 gu=copies([(wg_hbm, wg_v), (wu_hbm, wu_v)]),
                 rest=copies([(wd_hbm, wd_v)] +
                             [(wo_hbm.at[:, lanes(c)], wo_v.at[c]) for c in range(NC)]))

    def run(actions):
        cost = 0
        for act, arg in actions:
            if act == "start":
                start(batch[arg])
            elif act == "wait":
                wait(batch[arg])
            elif act == "w":
                for p, i, g in steps[arg[0]][arg[1]:arg[2]]:
                    if i == 0:
                        jobs.append(prep_qkv(p, g))
                        cost += 700
            else:
                job, c = dict(x=(prep_x, 800), router=(router, 1200), wo=(prep_wo, 1000),
                              route=(route, 100), hidden=(ffn_hidden, 0), out=(ffn_out, 0))[act]
                (slow if act in ("hidden", "out") else jobs).append(job(*arg))
                cost += c
        return cost

    for actions, budget in HEAD:
        run(actions)
        background(budget)
    for s, work in enumerate(steps):
        cost = 0 if s else 600
        for t in range(NU):
            cost += run(EVENTS.get((s, t), ()))
            project(work, t)
            share = cost / (NU - t)
            background(share)
            cost -= share
            background(FFN_BUDGET.get(s, 0) / NU, slow)
        background(1e9)
        for p, i, g in work:
            if p == 1:
                softmax(i, g)
    for i in range(NB):
        for cs, us in (LAST_PIECES if i == NB - 1 else OUT_PIECES):
            tiles = out_proj(i, cs, us)
            background(1e9, slow)
            mix(i, tiles)
    wait([cp_out(i, c) for i in range(NB) for c in range(NC)])


@jax.jit
def pallas_gated_mix__sliding_local_dilated__moe_arch_mod__prompt_kernel(
    A_x: jax.Array,
    A_wqkv: jax.Array,
    A_wo: jax.Array,
    B_x: jax.Array,
    B_w_r: jax.Array,
    B_w_gate: jax.Array,
    B_w_up: jax.Array,
    B_w_down: jax.Array,
    gate_w: jax.Array,
):
    hbm = pl.BlockSpec(memory_space=pl.ANY)
    return pl.pallas_call(
        _kernel,
        out_shape=jax.ShapeDtypeStruct((S, D), A_x.dtype),
        in_specs=[hbm] * 8,
        out_specs=hbm,
        scratch_shapes=[
            pltpu.VMEM((NC, S // 2, 128), u32),
            pltpu.VMEM((D // 2, 3 * D), u32),
            pltpu.VMEM((NC, D // 2, 128), u32),
            pltpu.VMEM((F // 2, D), u32),
            pltpu.VMEM((F // 2, D), u32),
            pltpu.VMEM((F // 2, D), u32),
            pltpu.VMEM((NC, S // 2, 128), u32),
            pltpu.VMEM((NC, 3 * D, 128), f32),
            pltpu.VMEM((NB * NU, 128), f32),
            pltpu.VMEM((D,), bf16),
            pltpu.VMEM((D,), bf16),
            pltpu.SemaphoreType.DMA((N_SEMS,)),
        ],
        compiler_params=pltpu.CompilerParams(
            vmem_limit_bytes=100 * 1024 * 1024),
    )(A_x.reshape(S, D), A_wqkv, A_wo, B_w_r, B_w_gate.T, B_w_up.T, B_w_down,
      gate_w).reshape(A_x.shape)
```

```python
import functools
import itertools
import math

import jax
import jax.numpy as jnp
from jax import lax
import jax.experimental.pallas as pl
import jax.experimental.pallas.tpu as pltpu

S, D, H, F = 2048, 640, 32, 1728
DH = D // H
W = 8
HG = H // 8
GR = 8 * DH
TB = 512
NB = S // TB
NU = TB // 128
NC = D // 128
NE = W - 1
N_SEMS = 10
SCALE = DH ** -0.5
EXP_SCALE = SCALE * math.log2(math.e)
MASKED = -1e9 / SCALE

HEAD = (
    ([("start", "w0"), ("start", "x0"), ("wait", "w0"), ("start", "w1"), ("w", (0, 0, 3))], 1e9),
    ([("wait", "x0"), ("start", "w2"), ("x", (0,))], 201),
)
EVENTS = {
    (0, 1): [("wait", "w1"), ("start", "w3"), ("w", (1, 0, 3))],
    (1, 0): [("w", (2, 0, 3))],
    (2, 1): [("wait", "w2"), ("start", "x1"), ("w", (3, 0, 3))],
    (3, 0): [("w", (4, 0, 3)), ("w", (5, 0, 3))],
    (4, 0): [("wait", "w3"), ("start", "x2"), ("w", (6, 0, 1))],
    (5, 0): [("w", (6, 1, 3))],
    (6, 0): [("wait", "x1"), ("w", (7, 0, 3)), ("x", (1,))],
    (7, 0): [("wait", "x2"), ("start", "gu"), ("start", "rest"), ("w", (8, 0, 3))],
    (8, 0): [("router", (0,)), ("router", (1,))],
    (9, 0): [("router", (2,))],
    (10, 0): [("x", (2,))],
    (11, 0): [("router", (3,))],
    (12, 0): [("route", ())],
    (13, 0): [("wait", "gu"), ("wait", "rest"), ("hidden", ()), ("out", ())],
    (14, 0): [("x", (3,))],
    (17, 0): [("wo", ())],
}
FFN_BUDGET = {13: 3600, 14: 3200, 15: 3600, 16: 3600, 17: 3200, 18: 3000}
OUT_PIECES = [((0, 1, 2, 3, 4), (0, 1)), ((0, 1, 2, 3, 4), (2, 3))]
LAST_PIECES = [((0, 1, 2), (0, 1)), ((0, 1, 2), (2, 3)), ((3,), (0, 1, 2, 3)),
               ((4,), (0, 1)), ((4,), (2,)), ((4,), (3,))]

f32, bf16, u32 = jnp.float32, jnp.bfloat16, jnp.uint32


def _kernel(x_hbm, wqkv_hbm, wo_hbm, wr_hbm, wg_hbm, wu_hbm, wd_hbm, gw_hbm,
            out_hbm,
            x_v, wqkv_v, wo_v, wg_v, wu_v, wd_v, out_v,
            tmp, score_s, wr_ref, gw_ref, sems):
    free_sems = iter(range(1, N_SEMS))

    def copies(pairs):
        sem = sems.at[next(free_sems)]
        return [pltpu.make_async_copy(src, dst, sem) for src, dst in pairs]

    def start(cps):
        for c in cps:
            c.start()

    def wait(cps):
        for c in cps:
            c.wait()

    def rows(i):
        return pl.ds(pl.multiple_of(i * (TB // 2), TB // 2), TB // 2)

    def lanes(c):
        return pl.ds(c * 128, 128)

    x_hbm, out_hbm, wqkv_hbm, wo_hbm, wg_hbm, wu_hbm, wd_hbm = (
        r.bitcast(u32) for r in (x_hbm, out_hbm, wqkv_hbm, wo_hbm, wg_hbm, wu_hbm, wd_hbm))

    def cp_x(lo, hi, extra=()):
        rws = pl.ds(lo * (TB // 2), (hi - lo) * (TB // 2))
        return copies([(x_hbm.at[rws, lanes(c)], x_v.at[c, rws]) for c in range(NC)] + list(extra))

    def cp_out(i, c):
        return pltpu.make_async_copy(out_v.at[c, rows(i)], out_hbm.at[rows(i), lanes(c)],
                                     sems.at[0])

    def slab(i, u):
        return pl.ds(i * (TB // 2) + u, 64, stride=NU)

    def load_rows(ref, rws=slice(None)):
        return jnp.concatenate([ref[c, rws, :] for c in range(ref.shape[0])], axis=1)

    def load_bf16(ref, rws=slice(None)):
        return pltpu.bitcast(load_rows(ref, rws), bf16)

    def store_bf16(ref, rws, val):
        val = pltpu.bitcast(val.astype(bf16), u32)
        for c in range(ref.shape[0]):
            ref[c, rws, :] = val[:, c * 128:(c + 1) * 128]

    def head_major_rows(base, d):
        return pl.ds(base + d, 8, stride=DH)

    wT, woT, xT, gate, oT = {}, {}, {}, {}, {}
    w_ready = set()

    def prep_qkv(p, g):
        base = p * D + g * GR
        for t in range(base // 128, (base + GR - 1) // 128 + 1):
            if t not in w_ready:
                w_ready.add(t)
                for c in range(NC):
                    tmp[c, lanes(t), :] = pltpu.bitcast(
                        wqkv_v[pl.ds(c * 64, 64), lanes(t)], bf16).astype(f32).T
                    yield 60
        parts = []
        for d in range(0, DH, 2):
            two = jnp.concatenate([load_rows(tmp, head_major_rows(base, d)),
                                   load_rows(tmp, head_major_rows(base, d + 1))], axis=0)
            parts.append(two.astype(bf16))
            yield 30
        wT[p, g] = jnp.concatenate(parts, axis=0)

    def prep_wo():
        for c in range(NC):
            perm = jnp.concatenate(
                [wo_v[c, pl.ds(g * GR // 2 + dp, 8, stride=DH // 2), :]
                 for g in range(HG) for dp in range(DH // 2)], axis=0)
            woT[c] = pltpu.bitcast(perm, bf16).T
            yield 200

    def prep_x(i):
        for u in range(NU):
            cols = []
            for c in range(NC):
                cols.append(pltpu.bitcast(x_v[c, slab(i, u), :], bf16).T)
            xT[i, u] = jnp.concatenate(cols, axis=0)
            yield 201

    def router(i):
        wr = wr_ref[...].astype(f32).reshape(1, D)
        for u in range(NU):
            acc_r = None
            for c in range(NC):
                xs = pltpu.bitcast(x_v[c, slab(i, u), :], bf16).astype(f32)
                term = xs * wr[:, c * 128:(c + 1) * 128]
                acc_r = term if c == 0 else acc_r + term
                yield 50
            score_s[pl.ds(i * NU + u, 1), :] = jnp.sum(acc_r.T, axis=0, keepdims=True)
            yield 50

    lane = lax.broadcasted_iota(jnp.int32, (1, 128), 1)
    query, raw, logit, prob, inv, acc = {}, {}, {}, {}, {}, {}

    def taps(p, i, g, t, d, cur):
        prev = raw.pop((p, g, t, d)) if i > 0 else 0.0
        if i + 1 < NB:
            raw[p, g, t, d] = cur
        for wrap in range((W - 1 + NU - 1) // NU + 1):
            us = [u for u in range(NU) if 0 <= u - t + wrap * NU < W]
            if us:
                x = cur if wrap == 0 else pltpu.roll(
                    jnp.where(lane >= 128 - 2 * wrap, prev, cur), 2 * wrap, 1)
                for u in us:
                    yield u, u - t + wrap * NU, x

    def scores(i, g, t, k):
        for d in range(DH):
            for u, w, x in taps(1, i, g, t, d, k[d * 8:(d + 1) * 8]):
                term = query[i, g, u][d * 8:(d + 1) * 8] * x
                logit[u, w] = logit[u, w] + term if d else term

    def softmax(i, g):
        for u in range(NU):
            ls = []
            for w in range(W):
                l = logit.pop((u, w))
                if i == 0 and w > u:
                    l = jnp.where(lane >= 2 * ((w - u + NU - 1) // NU), l, MASKED)
                ls.append(l)
            m = functools.reduce(jnp.maximum, ls)
            for w in range(W):
                prob[u, w] = jnp.exp2((ls[w] - m) * EXP_SCALE)
            inv[u] = 1.0 / functools.reduce(jnp.add, [prob[u, w] for w in range(W)])

    def values(i, g, t, v):
        for d in range(DH):
            for u, w, x in taps(2, i, g, t, d, v[d * 8:(d + 1) * 8]):
                term = prob[u, w] * x
                acc[u, d] = acc[u, d] + term if (u, d) in acc else term
            if t == NU - 1 and d % 2:
                for u in range(NU):
                    pair = [acc.pop((u, d - 1)) * inv[u], acc.pop((u, d)) * inv[u]]
                    oT.setdefault((i, u), []).append(pltpu.bitcast(
                        pltpu.pack_elementwise(pair, packed_dtype=bf16), u32))

    def project(work, t):
        for i in sorted({i for _, i, _ in work}):
            mine = [(p, g) for p, ii, g in work if ii == i]
            lhs = [wT[pg] for pg in mine]
            if (0, 0) in mine:
                gw = gw_ref[...].astype(f32).reshape(1, D)
                lhs.append(jnp.broadcast_to(gw, (16, D)).astype(bf16))
            r = jnp.dot(jnp.concatenate(lhs, axis=0), xT[i, t], preferred_element_type=f32)
            if (0, 0) in mine:
                gt = jax.nn.sigmoid(r[len(mine) * GR:len(mine) * GR + 8])
                gate[i, t] = jnp.tile(gt, (16, 1)).T
            for n, (p, g) in enumerate(mine):
                part = r[n * GR:(n + 1) * GR]
                if p == 0:
                    query[i, g, t] = part
                else:
                    (scores, values)[p - 1](i, g, t, part)

    jobs, slow = [], []

    def background(budget, queue=jobs):
        while queue and budget > 0:
            cost = next(queue[0], None)
            if cost is None:
                queue.pop(0)
            else:
                budget -= cost

    picks = []

    def route():
        r = score_s[...]
        r = r.astype(bf16).astype(f32)
        key = jnp.where(r != r, -jnp.inf, r)
        sub = lax.broadcasted_iota(jnp.int32, (NB * NU, 128), 0)
        pos = (sub // NU) * TB + (lane // 2) * (2 * NU) + (sub % NU) * 2 + lane % 2
        free = pos >= 0
        for _ in range(2):
            m = jnp.max(jnp.where(free, key, -jnp.inf), keepdims=True)
            idx = jnp.min(jnp.where(free & (key == m), pos, S - 1))
            score = jnp.sum(jnp.where(pos == idx, r, 0.0), keepdims=True)
            free = free & (pos != idx)
            picks.append((idx, jax.nn.sigmoid(score)))
            yield 50

    row = lax.broadcasted_iota(jnp.int32, (16, D), 0)
    hidden = []

    def halves(ref, j):
        word = ref[pl.ds(8 * j, 8), :]
        return [pltpu.unpack_elementwise(word, index=n, packed_dtype=bf16, unpacked_dtype=f32)
                for n in range(2)]

    def picked(idx):
        tile = pl.ds(pl.multiple_of((idx // 16) * 8, 8), 8)
        return tile, row == idx % 16, load_bf16(x_v, tile).astype(f32)

    def ffn_hidden():
        xs = []
        for idx, _ in picks:
            _, hit, cur = picked(idx)
            xs.append(jnp.broadcast_to(
                jnp.sum(jnp.where(hit, cur, 0.0), axis=0, keepdims=True), (8, D)))

        def matvec(w, x):
            prod = w * x
            part = functools.reduce(
                jnp.add, [prod[:, c * 128:(c + 1) * 128] for c in range(NC)])
            return jnp.sum(part, axis=1, keepdims=True)

        for j in range(F // 16):
            hs = []
            for wg, wu in zip(halves(wg_v, j), halves(wu_v, j)):
                for x in xs:
                    half = 0.5 * matvec(wg, x)
                    h = (half * jnp.tanh(half) + half) * matvec(wu, x)
                    hs.append(jnp.broadcast_to(h, (8, 128)))
            hidden.append(hs)
            yield 130

    def ffn_out():
        ys = [None] * len(picks)
        for j in range(F // 16):
            for n, wd in enumerate(halves(wd_v, j)):
                for k in range(len(picks)):
                    term = wd * jnp.tile(hidden[j][n * len(picks) + k], (1, NC))
                    ys[k] = term if ys[k] is None else ys[k] + term
            yield 50
        assert len(xT) == NB * NU
        for (idx, weight), y in zip(picks, ys):
            tile, hit, cur = picked(idx)
            y = jnp.sum(y, axis=0, keepdims=True) * weight
            store_bf16(x_v, tile, jnp.where(hit, cur + y, cur))

    def out_proj(i, cs, us):
        rhs = jnp.concatenate(
            [pltpu.bitcast(jnp.concatenate(oT[i, u], axis=0), bf16) for u in us], axis=1)
        aT = jnp.dot(jnp.concatenate([woT[c] for c in cs], axis=0), rhs,
                     preferred_element_type=f32)
        return {(c, u): aT[n * 128:(n + 1) * 128, m * 128:(m + 1) * 128]
                for n, c in enumerate(cs) for m, u in enumerate(us)}

    def mix(i, tiles):
        for (c, u), aT in tiles.items():
            b = pltpu.bitcast(x_v[c, slab(i, u), :], bf16).astype(f32)
            o = gate[i, u] * aT.T + (1.0 - gate[i, u]) * b
            out_v[c, slab(i, u), :] = pltpu.bitcast(o.astype(bf16), u32)
            if u == NU - 1 and i == NB - 1:
                cp_out(i, c).start()
            elif (u, c) == (NU - 1, NC - 1):
                start([cp_out(i, n) for n in range(NC)])

    n_groups = NB * HG
    steps = [[(p, n // HG, n % HG) for p, n in ((1, s), (2, s - 1), (0, s + 1))
              if 0 <= n < n_groups]
             for s in range(-1, n_groups + 1)]
    steps[:3] = [[item] for work in steps[:3] for item in sorted(work, reverse=True)]

    def w_tiles(work):
        return [t for p, i, g in work
                for t in range((p * D + g * GR) // 128, (p * D + g * GR + GR - 1) // 128 + 1)]

    seen = set()

    def w_pairs(lo, hi):
        new = [t for work in steps[lo:hi] for t in w_tiles(work)]
        new = [t for t in dict.fromkeys(new) if t not in seen]
        seen.update(new)
        runs = [[t for _, t in run] for _, run in
                itertools.groupby(enumerate(sorted(new)), lambda nt: nt[1] - nt[0])]
        cols = [pl.ds(run[0] * 128, len(run) * 128) for run in runs]
        return [(wqkv_hbm.at[:, cl], wqkv_v.at[:, cl]) for cl in cols]

    batch = dict(w0=copies(w_pairs(0, 1)), w1=copies(w_pairs(1, 3)), w2=copies(w_pairs(3, 6)),
                 w3=copies(w_pairs(6, 7)),
                 x0=cp_x(0, 1, [(gw_hbm, gw_ref), (wr_hbm, wr_ref)]),
                 x1=cp_x(1, 2, w_pairs(7, len(steps))), x2=cp_x(2, NB),
                 gu=copies([(wg_hbm, wg_v), (wu_hbm, wu_v)]),
                 rest=copies([(wd_hbm, wd_v)] +
                             [(wo_hbm.at[:, lanes(c)], wo_v.at[c]) for c in range(NC)]))

    def run(actions):
        cost = 0
        for act, arg in actions:
            if act == "start":
                start(batch[arg])
            elif act == "wait":
                wait(batch[arg])
            elif act == "w":
                for p, i, g in steps[arg[0]][arg[1]:arg[2]]:
                    if i == 0:
                        jobs.append(prep_qkv(p, g))
                        cost += 700
            else:
                job, c = dict(x=(prep_x, 800), router=(router, 1200), wo=(prep_wo, 1000),
                              route=(route, 100), hidden=(ffn_hidden, 0), out=(ffn_out, 0))[act]
                (slow if act in ("hidden", "out") else jobs).append(job(*arg))
                cost += c
        return cost

    for actions, budget in HEAD:
        run(actions)
        background(budget)
    for s, work in enumerate(steps):
        cost = 0 if s else 600
        for t in range(NU):
            cost += run(EVENTS.get((s, t), ()))
            project(work, t)
            share = cost / (NU - t)
            background(share)
            cost -= share
            background(FFN_BUDGET.get(s, 0) / NU, slow)
        background(1e9)
        for p, i, g in work:
            if p == 1:
                softmax(i, g)
    for i in range(NB):
        for cs, us in (LAST_PIECES if i == NB - 1 else OUT_PIECES):
            tiles = out_proj(i, cs, us)
            background(1e9, slow)
            mix(i, tiles)
    wait([cp_out(i, c) for i in range(NB) for c in range(NC)])


@jax.jit
def pallas_gated_mix__sliding_local_dilated__moe_arch_mod__prompt_kernel(
    A_x: jax.Array,
    A_wqkv: jax.Array,
    A_wo: jax.Array,
    B_x: jax.Array,
    B_w_r: jax.Array,
    B_w_gate: jax.Array,
    B_w_up: jax.Array,
    B_w_down: jax.Array,
    gate_w: jax.Array,
):
    hbm = pl.BlockSpec(memory_space=pl.ANY)
    return pl.pallas_call(
        _kernel,
        out_shape=jax.ShapeDtypeStruct((S, D), A_x.dtype),
        in_specs=[hbm] * 8,
        out_specs=hbm,
        scratch_shapes=[
            pltpu.VMEM((NC, S // 2, 128), u32),
            pltpu.VMEM((D // 2, 3 * D), u32),
            pltpu.VMEM((NC, D // 2, 128), u32),
            pltpu.VMEM((F // 2, D), u32),
            pltpu.VMEM((F // 2, D), u32),
            pltpu.VMEM((F // 2, D), u32),
            pltpu.VMEM((NC, S // 2, 128), u32),
            pltpu.VMEM((NC, 3 * D, 128), f32),
            pltpu.VMEM((NB * NU, 128), f32),
            pltpu.VMEM((D,), bf16),
            pltpu.VMEM((D,), bf16),
            pltpu.SemaphoreType.DMA((N_SEMS,)),
        ],
        compiler_params=pltpu.CompilerParams(
            vmem_limit_bytes=100 * 1024 * 1024),
    )(A_x.reshape(S, D), A_wqkv, A_wo, B_w_r, B_w_gate.T, B_w_up.T, B_w_down,
      gate_w).reshape(A_x.shape)
```
